```python
import jax
import jax.numpy as jnp

def _softmax(x, axis=-1):
    return jax.nn.softmax(x, axis=axis)

def _gelu(x):
    return jax.nn.gelu(x, approximate=True)

def _silu(x):
    return jax.nn.silu(x)

def _sigmoid(x):
    return jax.nn.sigmoid(x)

def _layernorm(x, axis=-1, eps=1e-05):
    m = jnp.mean(x, axis=axis, keepdims=True)
    v = jnp.var(x, axis=axis, keepdims=True)
    return (x - m) / jnp.sqrt(v + eps)

def _scatter_add(tgt, idx, src, axis=0):
    return tgt.at[idx].add(src)

def _segment_sum(src, seg, n):
    return jax.ops.segment_sum(src, seg, n)

class _Rng:

    def __init__(self, key):
        self._k = key

    def _next(self):
        self._k, sub = jax.random.split(self._k)
        return sub

    def normal(self, shape):
        return jax.random.normal(self._next(), shape, dtype=jnp.bfloat16)

    def randint(self, lo, hi, shape):
        return jax.random.randint(self._next(), shape, lo, hi, dtype=jnp.int32)

    def uniform(self, shape, lo=0.0, hi=1.0):
        return jax.random.uniform(self._next(), shape, jnp.bfloat16, lo, hi)

    def permutation(self, n):
        return jax.random.permutation(self._next(), n)
kernel_name = 'adaLN_cond__memory_aug_infini_attn__dense_activation_gelu__prompt'

def _fwd_setup_inputs():
    _rng = _Rng(jax.random.key(int.from_bytes(__import__("os").urandom(4), "little")))
    _w = lambda a: (lambda t: t.astype(jnp.bfloat16) if jnp.issubdtype(t.dtype, jnp.floating) else t)(jnp.asarray(a))

    def _A_setup():
        B, S, D, H = (1, 2048, 640, 32)
        N = 4
        L = max(1, S // N)
        sc = D ** (-0.5)
        return {'x': _w((lambda *s: _rng.normal(s) * 0.05)(B, N * L, D)), 'wq': _w((lambda *s: _rng.normal(s) * 0.05)(D, D) * sc), 'wk': _w((lambda *s: _rng.normal(s) * 0.05)(D, D) * sc), 'wv': _w((lambda *s: _rng.normal(s) * 0.05)(D, D) * sc), 'wo': _w((lambda *s: _rng.normal(s) * 0.05)(D, D) * sc), 'beta': _w((lambda *s: _rng.normal(s) * 0.05)(H))}
    _A_in = _A_setup()

    def _B_setup():
        B, S, D, F = (1, 2048, 640, 1728)
        return {'x': _w((lambda *s: _rng.normal(s) * 0.05)(B, S, D)), 'w1': _w((lambda *s: _rng.normal(s) * 0.05)(D, F) * D ** (-0.5)), 'b1': _w((lambda *s: _rng.normal(s) * 0.05)(F) * 0.01), 'w2': _w((lambda *s: _rng.normal(s) * 0.05)(F, D) * F ** (-0.5)), 'b2': _w((lambda *s: _rng.normal(s) * 0.05)(D) * 0.01)}
    _B_in = _B_setup()
    return {'A_x': _A_in['x'], 'A_wq': _A_in['wq'], 'A_wk': _A_in['wk'], 'A_wv': _A_in['wv'], 'A_wo': _A_in['wo'], 'A_beta': _A_in['beta'], 'B_x': _B_in['x'], 'B_w1': _B_in['w1'], 'B_b1': _B_in['b1'], 'B_w2': _B_in['w2'], 'B_b2': _B_in['b2'], 'c': _w((lambda *s: _rng.normal(s) * 0.05)(1, 640)), 'w_mod': _w((lambda *s: _rng.normal(s) * 0.05)(640, 6 * 640) * 640 ** (-0.5))}

def _fwd_reference(A_x, A_wq, A_wk, A_wv, A_wo, A_beta, B_x, B_w1, B_b1, B_w2, B_b2, c, w_mod):

    def _A_ref(x, wq, wk, wv, wo, beta):
        B, S, D = x.shape
        H = 32
        Dh = D // H
        N = 4
        L = S // N
        q = (lambda x, *d: x.transpose(*d))((x @ wq).reshape(B, S, H, Dh), 0, 2, 1, 3).reshape(B, H, N, L, Dh)
        k = (lambda x, *d: x.transpose(*d))((x @ wk).reshape(B, S, H, Dh), 0, 2, 1, 3).reshape(B, H, N, L, Dh)
        v = (lambda x, *d: x.transpose(*d))((x @ wv).reshape(B, S, H, Dh), 0, 2, 1, 3).reshape(B, H, N, L, Dh)
        phi = lambda t: jnp.where(t > 0, t + 1.0, jnp.exp(t))
        scale = Dh ** (-0.5)
        ar = jnp.arange(L)
        mask = (lambda x, dt: x.astype(dt))(ar[:, None] < ar[None, :], x.dtype) * -1000000000.0
        g = _sigmoid(beta).reshape(1, H, 1, 1)
        M = jnp.einsum('bhd,bhe->bhde', q[:, :, 0, 0, :] * 0.0, q[:, :, 0, 0, :] * 0.0)
        z = q[:, :, 0, 0, :] * 0.0
        outs = []
        for s in range(N):
            qs, ks, vs = (q[:, :, s].copy(), k[:, :, s].copy(), v[:, :, s].copy())
            logits = jnp.einsum('bhqd,bhkd->bhqk', qs, ks) * scale + mask
            p = _softmax(logits, axis=-1)
            a_dot = jnp.einsum('bhqk,bhkd->bhqd', p, vs)
            pq = phi(qs)
            num = jnp.einsum('bhld,bhde->bhle', pq, M)
            den = jnp.einsum('bhld,bhd->bhl', pq, z)[..., None] + 1e-06
            a_mem = num / den
            o = g * a_mem + (1.0 - g) * a_dot
            outs.append(o)
            pk = phi(ks)
            M = M + jnp.einsum('bhld,bhle->bhde', pk, vs)
            z = z + jnp.einsum('bhld->bhd', pk)
        o = (lambda x, *d: x.transpose(*d))(jnp.stack(outs, 2).reshape(B, H, S, Dh), 0, 2, 1, 3).reshape(B, S, D)
        return o @ wo

    def _B_ref(x, w1, b1, w2, b2):
        h = jnp.einsum('bsd,df->bsf', x, w1) + b1
        h = _gelu(h)
        return jnp.einsum('bsf,fd->bsd', h, w2) + b2
    x = A_x
    mod = (_silu(c) @ w_mod).reshape(c.shape[0], 6, 1, -1)
    sa, ca, ga, sb, cb, gb = (mod[:, 0].copy(), mod[:, 1].copy(), mod[:, 2].copy(), mod[:, 3].copy(), mod[:, 4].copy(), mod[:, 5].copy())
    h = _layernorm(x, axis=-1) * (1 + ca) + sa
    x = x + ga * _A_ref(h, A_wq, A_wk, A_wv, A_wo, A_beta)
    h = _layernorm(x, axis=-1) * (1 + cb) + sb
    x = x + gb * _B_ref(h, B_w1, B_b1, B_w2, B_b2)
    return x

def setup_inputs():
    _inp = _fwd_setup_inputs()
    _gk = jax.random.fold_in(jax.random.key(int.from_bytes(__import__("os").urandom(4), "little")), 2 ** 31 - 1)
    _shapes = [[1, 2048, 640]]
    _dtypes = ['bfloat16']
    _gks = jax.random.split(_gk, len(_shapes))
    _gs = [jax.random.normal(k, s, dtype=jnp.dtype(d)) * 0.05 for k, s, d in zip(_gks, _shapes, _dtypes)]
    _inp['grad_out'] = _gs[0]
    return _inp

def reference(A_x, A_wq, A_wk, A_wv, A_wo, A_beta, B_w1, B_b1, B_w2, B_b2, c, w_mod, B_x, grad_out):
    _const = dict(B_x=B_x)

    def _f(*_d):
        return _fwd_reference(**{'A_x': _d[0], 'A_wq': _d[1], 'A_wk': _d[2], 'A_wv': _d[3], 'A_wo': _d[4], 'A_beta': _d[5], 'B_w1': _d[6], 'B_b1': _d[7], 'B_w2': _d[8], 'B_b2': _d[9], 'c': _d[10], 'w_mod': _d[11], **_const})
    _out, _vjp = jax.vjp(_f, A_x, A_wq, A_wk, A_wv, A_wo, A_beta, B_w1, B_b1, B_w2, B_b2, c, w_mod)
    _grads = _vjp(grad_out)
    _out0 = jnp.asarray(_out)
    return (_out0, *[jnp.asarray(_g) for _g in _grads])
```

```python
import contextlib
import math

import jax
import jax.numpy as jnp
import jax.experimental.pallas as pl
import jax.experimental.pallas.tpu as pltpu

bf16 = jnp.bfloat16
f32 = jnp.float32
u32 = jnp.uint32

S, D, H, DH, NSEG, L, F = 2048, 640, 32, 20, 4, 512, 1728
FP = 1792
NQ = 8
QR = 80
FCH = 288
NFC = F // FCH
SCALE = DH ** -0.5
LOG2E = math.log2(math.e)
GELU_C1 = math.sqrt(2.0 / math.pi)
GELU_C2 = GELU_C1 * 0.044715
EPS = 1e-5
POFF = (0, 64, 192, 384)

_PROFILE = False


def _scope(name):
    return jax.named_scope(name) if _PROFILE else contextlib.nullcontext()


NN = (((1,), (0,)), ((), ()))
NT = (((1,), (1,)), ((), ()))


def _dot(a, b, dims):
    return jax.lax.dot_general(a, b, dims, preferred_element_type=f32)


def _B(x):
    return pltpu.bitcast(x, bf16)


def _U(x):
    return pltpu.bitcast(x, u32)


def _pack(x):
    return _U(x.astype(bf16))


def _iota(shape, dim):
    return jax.lax.broadcasted_iota(jnp.int32, shape, dim)


def _rep(p, n=L):
    return jnp.concatenate([p] * (n // 128), axis=1)


def _fold(x):
    acc = x[:, 0:128]
    for t in range(1, x.shape[1] // 128):
        acc = acc + x[:, t * 128:(t + 1) * 128]
    return acc


def _colrep(row):
    return jnp.broadcast_to(row, (128, row.shape[1])).T


def _rowsum(acc):
    return jnp.sum(acc.T, axis=0, keepdims=True)


def _phi(x):
    return jnp.where(x > 0, x + 1.0, jnp.exp(x))


def _mo(x, m):
    return pl.multiple_of(x, m)


def _assemble(w):
    lo = _iota((8, w[0].shape[1]), 0) < 4
    return jnp.concatenate([
        w[0][0:16], jnp.where(lo, w[0][16:24], w[1][0:8]), w[1][8:24],
        w[2][8:24], jnp.where(lo, w[2][24:32], w[3][8:16]), w[3][16:32]], axis=0)


def _assemble_rows(r):
    lo = _iota(r[0].shape, 0) < 4
    return jnp.concatenate([
        r[0], r[0], jnp.where(lo, r[0], r[1]), r[1], r[1],
        r[2], r[2], jnp.where(lo, r[2], r[3]), r[3], r[3]], axis=0)


def _head_partials(x):
    lo = _iota((8, x.shape[1]), 0) < 4
    v = [x[8 * k:8 * k + 8] for k in range(10)]
    return [v[0] + v[1] + jnp.where(lo, v[2], 0.0),
            jnp.where(lo, 0.0, v[2]) + v[3] + v[4],
            v[5] + v[6] + jnp.where(lo, v[7], 0.0),
            jnp.where(lo, 0.0, v[7]) + v[8] + v[9]]


def _kernel(x_hbm, wq_hbm, wk_hbm, wv_hbm, wo_hbm, beta_hbm, w1_hbm, b1_hbm, w2_hbm, b2_hbm,
            c_hbm, wmod_hbm, dy_hbm,
            out_hbm, dx_hbm, dwq_hbm, dwk_hbm, dwv_hbm, dwo_hbm, dbeta_hbm, dw1_hbm, db1_hbm,
            dw2_hbm, db2_hbm, dc_hbm, dwmod_hbm,
            x_buf, dy_buf, wqkv_buf, wo_buf, w1_buf, w2_buf, wmod_buf,
            beta_buf, b1_buf, b2_buf, c_buf,
            st_w1, st_w2, st_w,
            wqT, wkvT, woT, w1N, w2T,
            modT, b1T, b2T, gT_ref, scT, dsc_ref,
            xT, h1T, hnext, kT, vT, stat1, stat2,
            mt_state, m_state, dm_state, dmt_state,
            qT, qsT, pqT, knat, vnat, vaug, p_ref, sbuf,
            adot, amem, rden, cinv, oT, sA, sB, sC,
            h2T, dffnT, dyT, gactT, duT, dOp, dqkvT,
            acc_wqkv, acc_wo, acc_w1T, acc_w2, acc_vec, acc_b1,
            sems):
    def cp(src, dst, k):
        return pltpu.make_async_copy(src, dst, sems.at[k])

    def in_x(s):
        r = pl.ds(_mo(s * L, L), L)
        return cp(x_hbm.at[0, r, :], x_buf.at[r, :], 1 + s)

    in_wmodA = cp(wmod_hbm.at[:, pl.ds(0, 2 * D)], wmod_buf.at[:, pl.ds(0, 2 * D)], 0)
    in_w = [cp(w, wqkv_buf.at[k], 5 + k) for k, w in enumerate((wq_hbm, wk_hbm, wv_hbm))]
    in_wmodB = cp(wmod_hbm.at[:, pl.ds(2 * D, 4 * D)], wmod_buf.at[:, pl.ds(2 * D, 4 * D)], 8)
    in_wo = cp(wo_hbm, wo_buf, 9)
    in_w1 = cp(w1_hbm, w1_buf.at[pl.ds(0, F), :], 10)
    in_w2 = cp(w2_hbm, w2_buf.at[pl.ds(0, F), :], 11)
    in_dy = cp(dy_hbm.at[0], dy_buf, 12)
    in_small = [cp(c_hbm, c_buf, 21), cp(beta_hbm, beta_buf, 22), cp(b1_hbm, b1_buf, 23), cp(b2_hbm, b2_buf, 24)]

    for d in in_small:
        d.start()
    in_x(0).start()
    in_wmodA.start()
    in_w[1].start()
    in_w[2].start()
    in_x(1).start()
    in_w[0].start()
    in_wo.start()
    in_x(2).start()
    in_x(3).start()
    in_wmodB.start()
    in_dy.start()
    in_w1.start()
    in_w2.start()

    dm_state[...] = jnp.zeros(dm_state.shape, f32)
    dmt_state[...] = jnp.zeros(dmt_state.shape, f32)
    mt_state[0:NQ * 96, :] = jnp.zeros((NQ * 96, 128), f32)
    m_state[0:D, :] = jnp.zeros((D, 128), f32)
    gactT[F // 2:FP // 2, :] = jnp.zeros(((FP - F) // 2, L), u32)
    duT[F // 2:FP // 2, :] = jnp.zeros(((FP - F) // 2, L), u32)
    w1_buf[F:FP, :] = jnp.zeros((FP - F, D), bf16)
    w2_buf[F:FP, :] = jnp.zeros((FP - F, D), bf16)
    dsc_ref[...] = jnp.zeros(dsc_ref.shape, f32)

    for d in in_small:
        d.wait()

    def silu_parts():
        c = c_buf[...].astype(f32)
        sig_c = 1.0 / (1.0 + jnp.exp(-c))
        return c, sig_c

    def gate_row():
        beta = beta_buf[...].astype(f32).reshape(1, H)
        return 1.0 / (1.0 + jnp.exp(-beta))

    def head_onehot():
        return (_iota((D, H), 0) // DH) == _iota((D, H), 1)

    c, sig_c = silu_parts()
    sc = c * sig_c
    sc16 = jnp.broadcast_to(sc, (16, D)).astype(bf16)
    scT[...] = _colrep(sc.astype(bf16).astype(f32))

    def mod_chunks(lo, hi):
        for k in range(lo, hi):
            m = _dot(sc16, wmod_buf[:, k * D:(k + 1) * D], NN)[0:1, :]
            if k in (1, 4):
                m = m + 1.0
            modT[k * D:(k + 1) * D, :] = _colrep(m)

    def P(k, n=L):
        return _rep(modT[k * D:(k + 1) * D, :], n)

    bd80 = (_iota((QR, 128), 0) // DH) == (_iota((QR, 128), 1) // DH)
    lane80 = _iota((QR, 128), 1)
    bd = jnp.logical_and(bd80, lane80 < QR)
    mask2 = jnp.logical_or(bd, jnp.logical_and(
        jnp.logical_and(lane80 >= QR, lane80 < QR + 32),
        ((lane80 - QR) // 8) == (_iota((QR, 128), 0) // DH)))
    ONES_U = jnp.uint32(0x3F803F80)
    zeros24 = jnp.zeros((24, L), u32)
    ones24 = jnp.full((24, L), ONES_U, u32)

    b1row = b1_buf[...].astype(f32).reshape(1, F)
    for k in range(F // 128):
        b1T[k * 128:(k + 1) * 128, :] = _colrep(b1row[:, k * 128:(k + 1) * 128])
    b1T[F - 128:F, :] = _colrep(b1row[:, F - 128:F])
    b2T[...] = _colrep(b2_buf[...].astype(f32).reshape(1, D))
    gcol = jnp.sum(jnp.where(head_onehot(), jnp.broadcast_to(gate_row(), (D, H)), 0.0), axis=1, keepdims=True)
    gT_ref[...] = jnp.broadcast_to(gcol, (D, 128))

    def ln1_stats(s):
        r0 = _mo(s * (D // 2), 8)
        xt_b = x_buf[pl.ds(_mo(s * L, L), L), :].T
        xT[pl.ds(r0, D // 2), :] = _U(xt_b)
        xt = xt_b.astype(f32)
        mu = jnp.mean(xt, axis=0, keepdims=True)
        xc = xt - mu
        var = jnp.mean(xc * xc, axis=0, keepdims=True)
        rstd = jax.lax.rsqrt(var + EPS)
        stat1[pl.ds(_mo(s * 16, 8), 8), :] = jnp.broadcast_to(mu, (8, L))
        stat1[pl.ds(_mo(s * 16 + 8, 8), 8), :] = jnp.broadcast_to(rstd, (8, L))
        return xc * rstd

    in_x(0).wait()
    sA[...] = ln1_stats(0)
    in_wmodA.wait()
    mod_chunks(0, 2)
    hnext[...] = _pack(sA[...] * P(1) + P(0))
    in_w[1].wait()
    wkvT[0:D // 2, :] = _U(wqkv_buf[1].T)
    in_w[2].wait()
    wkvT[D // 2:D, :] = _U(wqkv_buf[2].T)

    def phase0(s, carry):
        @pl.when(s < NSEG - 1)
        def _():
            in_x(s + 1).wait()

        r0 = _mo(s * (D // 2), 8)
        h1T[pl.ds(r0, D // 2), :] = hnext[...]
        hb = _B(h1T[pl.ds(r0, D // 2), :])
        kk = _dot(_B(wkvT[0:D // 2, :]), hb, NN)
        kT[pl.ds(r0, D // 2), :] = _pack(kk)
        pqT[...] = _pack(_phi(kk))
        vv = _dot(_B(wkvT[D // 2:D, :]), hb, NN)
        vT[pl.ds(r0, D // 2), :] = _pack(vv)
        hnext[...] = _pack(ln1_stats(jnp.minimum(s + 1, NSEG - 1)) * P(1) + P(0))
        for acc in (acc_wqkv, acc_wo, acc_w1T, acc_w2, acc_vec, acc_b1):
            q = acc.shape[0] // NSEG
            acc[pl.ds(_mo(s * q, 8), q), :] = jnp.zeros((q, acc.shape[1]), f32)
        for i in range(NQ):
            pk_u = pqT[i * 40:(i + 1) * 40, :]
            v_u = vT[pl.ds(r0 + i * 40, 40), :]
            pk_w = _B(jnp.concatenate([pk_u, zeros24], axis=0))
            v_aug = jnp.concatenate([v_u, ones24], axis=0)
            mt = _dot(_B(v_aug[0:48]), pk_w, NT)
            mm = _dot(_B(pk_u), _B(v_aug), NT)
            a0 = _mo(s * (NQ * 96) + i * 96, 8)
            mt_state[pl.ds(a0 + NQ * 96, 96), :] = mt_state[pl.ds(a0, 96), :] + mt
            b0 = _mo(s * D + i * QR, 8)
            m_state[pl.ds(b0 + D, QR), :] = m_state[pl.ds(b0, QR), :] + mm
        return carry

    with _scope("phase0"):
        jax.lax.fori_loop(0, NSEG, phase0, 0)

    in_w[0].wait()
    in_wo.wait()
    in_wmodB.wait()
    wqT[...] = _U(wqkv_buf[0].T)
    woT[...] = _U(wo_buf[...].T)
    mod_chunks(2, 6)
    in_dy.wait()
    in_w1.wait()
    in_w2.wait()

    HL = L // 2

    def out_copy(s, hf):
        r = pl.ds(_mo(s * L + hf * HL, HL), HL)
        return cp(x_buf.at[r, :], out_hbm.at[0, r, :], 25 + 2 * s + hf)

    def dx_copy(s, hf):
        r = pl.ds(_mo(s * L + hf * HL, HL), HL)
        return cp(dy_buf.at[r, :], dx_hbm.at[0, r, :], 33 + 2 * s + hf)

    o_w1 = cp(st_w1, dw1_hbm, 0)
    o_w2 = cp(st_w2, dw2_hbm, 1)
    o_wo = cp(st_w.at[3], dwo_hbm, 2)
    o_w = [cp(st_w.at[k], dst, 3 + k) for k, dst in enumerate((dwq_hbm, dwk_hbm, dwv_hbm))]
    o_b1 = cp(b1_buf, db1_hbm, 12)
    o_b2 = cp(b2_buf, db2_hbm, 13)
    o_beta = cp(beta_buf, dbeta_hbm, 14)
    o_c = cp(c_buf, dc_hbm, 15)

    def o_mod(k):
        cs = pl.ds(_mo(k * D, 128), D)
        return cp(wmod_buf.at[:, cs], dwmod_hbm.at[:, cs], 6 + k)

    def dmod_chunk(k, c_):
        dm = _rowsum(acc_vec[pl.ds(_mo(k * D, 8), D), :])
        cs = pl.ds(_mo(k * D, 128), D)
        dsc_ref[...] += _dot(jnp.broadcast_to(dm, (16, D)).astype(bf16), wmod_buf[:, cs], NT)
        wmod_buf[:, cs] = (_rep(scT[...], D) * dm).astype(bf16)
        o_mod(k).start()
        return c_

    r40 = _iota((40, 128), 0)
    hmask = [jnp.logical_and(r40 >= 10 * j, r40 < 10 * j + 10) for j in range(4)]

    def segment(it, carry):
        s = NSEG - 1 - it
        r0 = _mo(s * (D // 2), 8)
        tok = pl.ds(_mo(s * L, L), L)
        last = it == NSEG - 1

        hb = _B(h1T[pl.ds(r0, D // 2), :])
        q = _dot(_B(wqT[...]), hb, NN)
        qT[...] = _pack(q)
        qsT[...] = _pack(q * (SCALE * LOG2E))
        pqT[...] = _pack(_phi(q))
        r16 = _iota((16, L), 0)
        for i in range(NQ):
            k_u = kT[pl.ds(r0 + i * 40, 40), :]
            v_u = vT[pl.ds(r0 + i * 40, 40), :]
            knat[i * 256:(i + 1) * 256, :] = _U(_B(jnp.concatenate([k_u, zeros24], axis=0)).T)
            vnat[i * 256:(i + 1) * 256, :] = _U(_B(jnp.concatenate([v_u, ones24], axis=0)).T)
            for j in range(4):
                keep = jnp.logical_and(r16 >= 2 * j, r16 < 2 * j + 10)
                vaug[(4 * i + j) * 16:(4 * i + j + 1) * 16, :] = jnp.where(keep, v_u[8 * j:8 * j + 16], ONES_U)

        def s_weights(i, t):
            qt = qsT[pl.ds(_mo(i * 40, 8), 40), t * 128:(t + 1) * 128]
            wq = jnp.concatenate([jnp.where(hmask[j], qt, jnp.uint32(0)) for j in range(4)], axis=1)
            return _B(jnp.concatenate([wq, zeros24], axis=0))

        def s_tile(i, t, u, mx):
            sc_ = _dot(_B(knat[pl.ds(_mo(i * 256 + u * 64, 8), 64), :]), s_weights(i, t), NN)
            if u == t:
                causal = _iota((128, 128), 0) <= _iota((128, 128), 1)
                sc_ = jnp.concatenate([jnp.where(causal, sc_[:, j * 128:(j + 1) * 128], -1e30)
                                       for j in range(4)], axis=1)
            sbuf[2 * POFF[t] + u * 128:2 * POFF[t] + (u + 1) * 128, :] = sc_
            for k in range(16):
                v = sc_[8 * k:8 * k + 8]
                mx = v if mx is None else jnp.maximum(mx, v)
            if u == t:
                mx = jnp.max(mx, axis=0, keepdims=True)
            return mx

        def p_tile(i, t, u, mx, ws):
            for j in range(4):
                lj = slice(j * 128, (j + 1) * 128)
                sj = sbuf[2 * POFF[t] + u * 128:2 * POFF[t] + (u + 1) * 128, lj]
                p = jnp.exp2(sj - mx[:, lj]).astype(bf16)
                p_ref[pl.ds(_mo(i * 640 + POFF[t] + u * 64, 8), 64), lj] = _U(p)
                va = _B(vaug[pl.ds(_mo((i * 4 + j) * 16, 16), 16), u * 128:(u + 1) * 128])
                w = _dot(va, p, NN)
                ws[j] = w if ws[j] is None else ws[j] + w
            if u == t:
                ls = [1.0 / (ws[j][24:32] if j < 2 else ws[j][0:8]) for j in range(4)]
                linv = _assemble_rows(ls)
                rq = pl.ds(_mo(i * QR, 8), QR)
                adot[rq, t * 128:(t + 1) * 128] = _assemble(ws) * linv
                cinv[rq, t * 128:(t + 1) * 128] = linv

        mx_first = None
        for u in range(4):
            mx_first = s_tile(0, 3, u, mx_first)

        def attn_fwd(i, mx3):
            i_next = jnp.minimum(i + 1, NQ - 1)
            mx = {3: mx3, 2: None, 1: None, 0: None, 4: None}
            ws = {t: [None] * 4 for t in range(4)}
            s_jobs = [(2, 0), (2, 1), (2, 2), (1, 0), (1, 1), (0, 0), (4, 0), (4, 1), (4, 2), (4, 3)]
            p_jobs = [(3, 0), (3, 1), (3, 2), (3, 3), (2, 0), (2, 1), (2, 2), (1, 0), (1, 1), (0, 0)]
            for (st, su), (pt, pu) in zip(s_jobs, p_jobs):
                if st == 4:
                    mx[4] = s_tile(i_next, 3, su, mx[4])
                else:
                    mx[st] = s_tile(i, st, su, mx[st])
                p_tile(i, pt, pu, mx[pt], ws[pt])
            rq = pl.ds(_mo(i * QR, 8), QR)
            mt = mt_state[pl.ds(_mo(s * (NQ * 96) + i * 96, 8), 96), :]
            z8 = mt[QR:QR + 8]
            zrep = jnp.concatenate([z8] * 10, axis=0)
            lhs = jnp.concatenate([jnp.where(bd, mt[0:QR], 0.0), jnp.where(bd, zrep, 0.0)], axis=0).astype(bf16)
            pq_w = _B(jnp.concatenate([pqT[pl.ds(_mo(i * 40, 8), 40), :], zeros24], axis=0))
            nd = _dot(lhs, pq_w, NN)
            rd = 1.0 / (nd[QR:] + 1e-6)
            am = nd[0:QR] * rd
            amem[rq, :] = am
            rden[rq, :] = rd
            g = _rep(gT_ref[rq, :])
            o = g * am + (1.0 - g) * adot[rq, :]
            oT[pl.ds(_mo(i * 40, 8), 40), :] = _pack(o)
            return mx[4]

        with _scope("attn_fwd"):
            jax.lax.fori_loop(0, NQ, attn_fwd, mx_first)

        attn = _dot(_B(woT[...]), _B(oT[...]), NN)
        sA[...] = attn
        x2 = _B(xT[pl.ds(r0, D // 2), :]).astype(f32) + P(2) * attn
        sB[...] = x2
        mu2 = jnp.mean(x2, axis=0, keepdims=True)
        xc2 = x2 - mu2
        var2 = jnp.mean(xc2 * xc2, axis=0, keepdims=True)
        rstd2 = jax.lax.rsqrt(var2 + EPS)
        xh2 = xc2 * rstd2
        sC[...] = xh2
        h2T[...] = _pack(xh2 * P(4) + P(3))
        stat2[...] = jnp.broadcast_to(rstd2, (8, L))
        dyT[...] = _U(dy_buf[tok, :].T)
        dffn = _B(dyT[...]).astype(f32) * P(5)
        dffnT[...] = _pack(dffn)
        acc_vec[6 * D:7 * D, :] += _fold(dffn)

        def ffn_chunk(ci, c_):
            rp = pl.ds(_mo(ci * (FCH // 2), 8), FCH // 2)
            rf = pl.ds(_mo(ci * FCH, 16), FCH)
            h2b = _B(h2T[...])
            dfb = _B(dffnT[...])
            u = _dot(w1_buf[rf, :], h2b, NN) + _rep(b1T[rf, :])
            dg = _dot(w2_buf[rf, :], dfb, NN)
            u2 = u * u
            th = jnp.tanh(u * (GELU_C1 + GELU_C2 * u2))
            hp = 0.5 * th + 0.5
            gactT[rp, :] = _pack(u * hp)
            gp = hp + (0.5 * u) * (1.0 - th * th) * (GELU_C1 + (3.0 * GELU_C2) * u2)
            du = dg * gp
            duT[rp, :] = _pack(du)
            acc_b1[rf, :] += _fold(du)
            a2 = acc_w2[rf, :] + _dot(_B(gactT[rp, :]), dfb, NT)
            acc_w2[rf, :] = a2
            st_w2[rf, :] = a2.astype(bf16)
            a1 = acc_w1T[rf, :] + _dot(_B(duT[rp, :]), h2b, NT)
            acc_w1T[rf, :] = a1
            st_w1[rf, :] = a1.astype(bf16)
            for blk in (ci, ci + NFC, jnp.minimum(ci + 2 * NFC, FP // 128 - 1)):
                rb = pl.ds(_mo(blk * 128, 128), 128)
                w1N[:, rb] = _U(w1_buf[rb, :].T)
                w2T[:, rb] = _U(w2_buf[rb, :].T)
            return c_

        with _scope("ffn_chunk"):
            jax.lax.fori_loop(0, NFC, ffn_chunk, 0)

        @pl.when(last)
        def _():
            o_w1.start()
            o_w2.start()

        def post_ffn(hf, c_):
            hl = pl.ds(_mo(hf * HL, HL), HL)
            rows = pl.ds(_mo(s * L + hf * HL, HL), HL)
            ffn = _dot(_B(w2T[...]), _B(gactT[:, hl]), NN) + _rep(b2T[...], HL)
            dyt = _B(dyT[:, hl]).astype(f32)
            acc_vec[5 * D:6 * D, :] += _fold(dyt * ffn)
            outT = sB[:, hl] + P(5, HL) * ffn
            x_buf[rows, :] = outT.astype(bf16).T
            dh2 = _dot(_B(w1N[...]), _B(duT[:, hl]), NN)
            xh2 = sC[:, hl]
            acc_vec[3 * D:4 * D, :] += _fold(dh2)
            acc_vec[4 * D:5 * D, :] += _fold(dh2 * xh2)
            dxh = dh2 * P(4, HL)
            m1 = jnp.mean(dxh, axis=0, keepdims=True)
            m2 = jnp.mean(dxh * xh2, axis=0, keepdims=True)
            dx2 = dyt + stat2[0:1, hl] * (dxh - m1 - xh2 * m2)
            sB[:, hl] = dx2
            acc_vec[2 * D:3 * D, :] += _fold(dx2 * sA[:, hl])
            dab = (dx2 * P(2, HL)).astype(bf16)
            sA[:, hl] = _dot(wo_buf[...], dab, NN)
            ao = acc_wo[...] + _dot(_B(oT[:, hl]), dab, NT)
            acc_wo[...] = ao
            st_w[3] = ao.astype(bf16)
            out_copy(s, hf).start()
            return c_

        with _scope("post_ffn"):
            jax.lax.fori_loop(0, 2, post_ffn, 0)

        @pl.when(last)
        def _():
            o_wo.start()
            jax.lax.fori_loop(2, 6, dmod_chunk, 0)
            b2_buf[...] = _rowsum(acc_vec[6 * D:7 * D, :]).reshape(D).astype(bf16)
            o_b2.start()
            parts = [_rowsum(acc_b1[k * 128:(k + 1) * 128, :]) for k in range(F // 128)]
            parts.append(_rowsum(acc_b1[F - 128:F, :])[:, 64:128])
            b1_buf[...] = jnp.concatenate(parts, axis=1).reshape(F).astype(bf16)
            o_b1.start()

        def attn_bwd(i, c_):
            rq = pl.ds(_mo(i * QR, 8), QR)
            rp = pl.ds(_mo(i * 40, 8), 40)
            do = sA[rq, :]
            ad = adot[rq, :]
            am = amem[rq, :]
            g = _rep(gT_ref[rq, :])
            acc_vec[pl.ds(_mo(7 * D + i * QR, 8), QR), :] += _fold(do * (am - ad))
            dop_b = (do * (1.0 - g) * cinv[rq, :]).astype(bf16)
            dOp[0:40, :] = _U(dop_b)
            parts = _head_partials(_B(dOp[0:40, :]).astype(f32) * ad)
            for j in range(4):
                hi = (-parts[j]).astype(bf16).astype(f32)
                lo = -parts[j] - hi
                dOp[40 + 8 * j:48 + 8 * j, :] = _pack(jnp.concatenate([hi, lo], axis=0))
            dnum = do * g * rden[rq, :]
            tp = _head_partials(dnum * am)
            wmem = jnp.concatenate([dnum] + [-x for x in tp] + [jnp.zeros((16, L), f32)], axis=0).astype(bf16)
            mm = m_state[pl.ds(_mo(s * D + i * QR, 8), QR), :]
            dpq = _dot(jnp.where(mask2, mm, 0.0).astype(bf16), wmem, NN)
            kk = _B(kT[pl.ds(r0 + i * 40, 40), :]).astype(f32)
            pk = _phi(kk)
            pk_w = jnp.concatenate([pk, jnp.zeros((48, L), f32)], axis=0).astype(bf16)
            v_aug = _B(jnp.concatenate([vT[pl.ds(r0 + i * 40, 40), :], ones24], axis=0))
            dms = dm_state[rq, :]
            dmts = dmt_state[rq, :]
            dpk = _dot(jnp.where(mask2, dms, 0.0).astype(bf16), v_aug, NN)
            dvm = _dot(jnp.where(bd, dmts, 0.0).astype(bf16), pk_w, NN)
            pq_u = pqT[rp, :]
            dm_state[rq, :] = dms + _dot(_B(pq_u), wmem, NT)
            dmt_state[rq, :] = dmts + _dot(dnum.astype(bf16), _B(jnp.concatenate([pq_u, zeros24], axis=0)), NT)
            qq = _B(qT[rp, :]).astype(f32)
            dq_mem = dpq * jnp.where(qq > 0, 1.0, _B(pq_u).astype(f32))
            dk_mem = dpk * jnp.where(kk > 0, 1.0, pk)

            dq = [[None] * 4 for _ in range(4)]
            dk = [[None] * 4 for _ in range(4)]
            dv = [[None] * 4 for _ in range(4)]

            def dp_tile(t, u):
                lt = slice(t * 128, (t + 1) * 128)
                dt = dOp[0:40, lt]
                wd = jnp.concatenate(
                    [jnp.concatenate([jnp.where(hmask[j], dt, jnp.uint32(0)), dOp[40 + 8 * j:48 + 8 * j, lt],
                                      jnp.zeros((16, 128), u32)], axis=0) for j in range(4)], axis=1)
                dp = _dot(_B(vnat[pl.ds(_mo(i * 256 + u * 64, 8), 64), :]), _B(wd), NN)
                res = []
                for j in range(4):
                    p = _B(p_ref[pl.ds(_mo(i * 640 + POFF[t] + u * 64, 8), 64), j * 128:(j + 1) * 128])
                    res.append((dp[:, j * 128:(j + 1) * 128] * p.astype(f32)).astype(bf16))
                return res

            def thin_tile(t, u, ds):
                lt = slice(t * 128, (t + 1) * 128)
                for j in range(4):
                    p = _B(p_ref[pl.ds(_mo(i * 640 + POFF[t] + u * 64, 8), 64), j * 128:(j + 1) * 128])
                    kw = _B(kT[pl.ds(r0 + i * 40 + 8 * j, 16), u * 128:(u + 1) * 128])
                    qw = _B(qT[pl.ds(_mo(i * 40 + 8 * j, 8), 16), lt])
                    dw = _B(dOp[8 * j:8 * j + 16, lt])
                    b = _dot(dw, p, NT)
                    a = _dot(qw, ds[j], NT)
                    e = _dot(kw, ds[j], NN)
                    dq[j][t] = e if dq[j][t] is None else dq[j][t] + e
                    dk[j][u] = a if dk[j][u] is None else dk[j][u] + a
                    dv[j][u] = b if dv[j][u] is None else dv[j][u] + b

            jobs = [(t, u) for t in (3, 2, 1, 0) for u in range(t + 1)]
            ds = dp_tile(*jobs[0])
            for n_, job in enumerate(jobs):
                ds_next = dp_tile(*jobs[n_ + 1]) if n_ + 1 < len(jobs) else None
                thin_tile(job[0], job[1], ds)
                ds = ds_next

            cat = lambda w: _assemble([jnp.concatenate(w[j], axis=1) for j in range(4)])
            dqkvT[rp, :] = _pack(cat(dq) * SCALE + dq_mem)
            dqkvT[pl.ds(_mo(D // 2 + i * 40, 8), 40), :] = _pack(cat(dk) * SCALE + dk_mem)
            dqkvT[pl.ds(_mo(D + i * 40, 8), 40), :] = _pack(cat(dv) + dvm)
            return c_

        with _scope("attn_bwd"):
            jax.lax.fori_loop(0, NQ, attn_bwd, 0)

        def qkv_bwd(hf, c_):
            hl = pl.ds(_mo(hf * HL, HL), HL)
            rows = pl.ds(_mo(s * L + hf * HL, HL), HL)
            dh1 = _dot(wqkv_buf[0], _B(dqkvT[0:D // 2, hl]), NN)
            dh1 = dh1 + _dot(wqkv_buf[1], _B(dqkvT[D // 2:D, hl]), NN)
            dh1 = dh1 + _dot(wqkv_buf[2], _B(dqkvT[D:3 * D // 2, hl]), NN)
            mu = stat1[pl.ds(_mo(s * 16, 8), 1), hl]
            rstd = stat1[pl.ds(_mo(s * 16 + 8, 8), 1), hl]
            xh1 = (_B(xT[pl.ds(r0, D // 2), hl]).astype(f32) - mu) * rstd
            acc_vec[0:D, :] += _fold(dh1)
            acc_vec[D:2 * D, :] += _fold(dh1 * xh1)
            dxh = dh1 * P(1, HL)
            m1 = jnp.mean(dxh, axis=0, keepdims=True)
            m2 = jnp.mean(dxh * xh1, axis=0, keepdims=True)
            dx = sB[:, hl] + rstd * (dxh - m1 - xh1 * m2)
            dy_buf[rows, :] = dx.astype(bf16).T
            dx_copy(s, hf).start()
            return c_

        with _scope("qkv_bwd"):
            jax.lax.fori_loop(0, 2, qkv_bwd, 0)

        @pl.when(last)
        def _():
            jax.lax.fori_loop(0, 2, dmod_chunk, 0)
            c_, sig = silu_parts()
            c_buf[...] = (dsc_ref[0:1, :] * (sig * (1.0 + c_ * (1.0 - sig)))).astype(bf16)
            o_c.start()
            gate = gate_row()
            dgc = jnp.sum(acc_vec[7 * D:8 * D, :], axis=1, keepdims=True)
            dgate = jnp.sum(jnp.where(head_onehot(), jnp.broadcast_to(dgc, (D, H)), 0.0), axis=0, keepdims=True)
            beta_buf[...] = (dgate * gate * (1.0 - gate)).reshape(H).astype(bf16)
            o_beta.start()

        def dw_qkv(k, c_):
            ra = pl.ds(_mo(k * D, 8), D)
            aw = acc_wqkv[ra, :] + _dot(_B(h1T[pl.ds(r0, D // 2), :]),
                                        _B(dqkvT[pl.ds(_mo(k * (D // 2), 8), D // 2), :]), NT)
            acc_wqkv[ra, :] = aw
            st_w[k] = aw.astype(bf16)
            for kk in range(3):
                @pl.when(jnp.logical_and(last, k == kk))
                def _():
                    o_w[kk].start()
            return c_

        with _scope("dw_qkv"):
            jax.lax.fori_loop(0, 3, dw_qkv, 0)
        return carry

    with _scope("segment"):
        jax.lax.fori_loop(0, NSEG, segment, 0)

    for s in range(NSEG):
        for hf in range(2):
            out_copy(s, hf).wait()
            dx_copy(s, hf).wait()
    for d in [o_w2, o_w1, o_wo, o_b1, o_b2, o_beta, o_c] + [o_mod(k) for k in range(6)] + o_w:
        d.wait()


@jax.jit
def pallas_adaLN_cond__memory_aug_infini_attn__dense_activation_gelu__prompt_kernel(
    A_x: jax.Array,
    A_wq: jax.Array,
    A_wk: jax.Array,
    A_wv: jax.Array,
    A_wo: jax.Array,
    A_beta: jax.Array,
    B_x: jax.Array,
    B_w1: jax.Array,
    B_b1: jax.Array,
    B_w2: jax.Array,
    B_b2: jax.Array,
    c: jax.Array,
    w_mod: jax.Array,
    grad_out: jax.Array,
):
    del B_x
    hbm = pl.BlockSpec(memory_space=pltpu.HBM)
    sds = jax.ShapeDtypeStruct
    V = pltpu.VMEM
    scratch = [
        V((S, D), bf16), V((S, D), bf16), V((3, D, D), bf16), V((D, D), bf16), V((FP, D), bf16),
        V((FP, D), bf16), V((D, 6 * D), bf16),
        V((H,), bf16), V((F,), bf16), V((D,), bf16), V((1, D), bf16),
        V((F, D), bf16), V((F, D), bf16), V((4, D, D), bf16),
        V((D // 2, D), u32), V((D, D), u32), V((D // 2, D), u32), V((D // 2, FP), u32), V((D // 2, FP), u32),
        V((6 * D, 128), f32), V((F, 128), f32), V((D, 128), f32), V((D, 128), f32), V((D, 128), f32),
        V((16, D), f32),
        V((NSEG * D // 2, L), u32), V((NSEG * D // 2, L), u32), V((D // 2, L), u32), V((NSEG * D // 2, L), u32),
        V((NSEG * D // 2, L), u32), V((NSEG * 16, L), f32), V((8, L), f32),
        V(((NSEG + 1) * NQ * 96, 128), f32), V(((NSEG + 1) * D, 128), f32), V((D, 128), f32), V((D, 128), f32),
        V((D // 2, L), u32), V((D // 2, L), u32), V((D // 2, L), u32),
        V((NQ * 256, 128), u32), V((NQ * 256, 128), u32), V((H * 16, L), u32), V((NQ * 640, L), u32), V((1280, L), f32),
        V((D, L), f32), V((D, L), f32), V((D, L), f32), V((D, L), f32), V((D // 2, L), u32),
        V((D, L), f32), V((D, L), f32), V((D, L), f32),
        V((D // 2, L), u32), V((D // 2, L), u32), V((D // 2, L), u32), V((FP // 2, L), u32), V((FP // 2, L), u32),
        V((72, L), u32), V((3 * D // 2, L), u32),
        V((3 * D, D), f32), V((D, D), f32), V((F, D), f32), V((F, D), f32), V((8 * D, 128), f32),
        V((F, 128), f32),
        pltpu.SemaphoreType.DMA((41,)),
    ]
    outs = pl.pallas_call(
        _kernel,
        in_specs=[hbm] * 13,
        out_specs=[hbm] * 13,
        out_shape=[
            sds((1, S, D), bf16), sds((1, S, D), bf16), sds((D, D), bf16), sds((D, D), bf16),
            sds((D, D), bf16), sds((D, D), bf16), sds((H,), bf16), sds((F, D), bf16), sds((F,), bf16),
            sds((F, D), bf16), sds((D,), bf16), sds((1, D), bf16), sds((D, 6 * D), bf16),
        ],
        scratch_shapes=scratch,
        compiler_params=pltpu.CompilerParams(vmem_limit_bytes=124 * 1024 * 1024),
    )(A_x, A_wq, A_wk, A_wv, A_wo, A_beta, B_w1.T, B_b1, B_w2, B_b2, c, w_mod, grad_out)
    out, dx, dwq, dwk, dwv, dwo, dbeta, dw1, db1, dw2, db2, dc, dwmod = outs
    return (out, dx, dwq, dwk, dwv, dwo, dbeta, dw1.T, db1, dw2, db2, dc, dwmod)
```

```python
import contextlib
import math

import jax
import jax.numpy as jnp
import jax.experimental.pallas as pl
import jax.experimental.pallas.tpu as pltpu

bf16 = jnp.bfloat16
f32 = jnp.float32
u32 = jnp.uint32

S, D, H, DH, NSEG, L, F = 2048, 640, 32, 20, 4, 512, 1728
FP = 1792
NQ = 8
QR = 80
FCH = 288
NFC = F // FCH
SCALE = DH ** -0.5
LOG2E = math.log2(math.e)
GELU_C1 = math.sqrt(2.0 / math.pi)
GELU_C2 = GELU_C1 * 0.044715
EPS = 1e-5
POFF = (0, 64, 192, 384)

_PROFILE = False


def _scope(name):
    return jax.named_scope(name) if _PROFILE else contextlib.nullcontext()


NN = (((1,), (0,)), ((), ()))
NT = (((1,), (1,)), ((), ()))


def _dot(a, b, dims):
    return jax.lax.dot_general(a, b, dims, preferred_element_type=f32)


def _B(x):
    return pltpu.bitcast(x, bf16)


def _U(x):
    return pltpu.bitcast(x, u32)


def _pack(x):
    return _U(x.astype(bf16))


def _iota(shape, dim):
    return jax.lax.broadcasted_iota(jnp.int32, shape, dim)


def _rep(p, n=L):
    return jnp.concatenate([p] * (n // 128), axis=1)


def _fold(x):
    acc = x[:, 0:128]
    for t in range(1, x.shape[1] // 128):
        acc = acc + x[:, t * 128:(t + 1) * 128]
    return acc


def _colrep(row):
    return jnp.broadcast_to(row, (128, row.shape[1])).T


def _rowsum(acc):
    return jnp.sum(acc.T, axis=0, keepdims=True)


def _phi(x):
    return jnp.where(x > 0, x + 1.0, jnp.exp(x))


def _mo(x, m):
    return pl.multiple_of(x, m)


def _assemble(w):
    lo = _iota((8, w[0].shape[1]), 0) < 4
    return jnp.concatenate([
        w[0][0:16], jnp.where(lo, w[0][16:24], w[1][0:8]), w[1][8:24],
        w[2][8:24], jnp.where(lo, w[2][24:32], w[3][8:16]), w[3][16:32]], axis=0)


def _assemble_rows(r):
    lo = _iota(r[0].shape, 0) < 4
    return jnp.concatenate([
        r[0], r[0], jnp.where(lo, r[0], r[1]), r[1], r[1],
        r[2], r[2], jnp.where(lo, r[2], r[3]), r[3], r[3]], axis=0)


def _head_partials(x):
    lo = _iota((8, x.shape[1]), 0) < 4
    v = [x[8 * k:8 * k + 8] for k in range(10)]
    return [v[0] + v[1] + jnp.where(lo, v[2], 0.0),
            jnp.where(lo, 0.0, v[2]) + v[3] + v[4],
            v[5] + v[6] + jnp.where(lo, v[7], 0.0),
            jnp.where(lo, 0.0, v[7]) + v[8] + v[9]]


def _kernel(x_hbm, wq_hbm, wk_hbm, wv_hbm, wo_hbm, beta_hbm, w1_hbm, b1_hbm, w2_hbm, b2_hbm,
            c_hbm, wmod_hbm, dy_hbm,
            out_hbm, dx_hbm, dwq_hbm, dwk_hbm, dwv_hbm, dwo_hbm, dbeta_hbm, dw1_hbm, db1_hbm,
            dw2_hbm, db2_hbm, dc_hbm, dwmod_hbm,
            x_buf, dy_buf, wqkv_buf, wo_buf, w1_buf, w2_buf, wmod_buf,
            beta_buf, b1_buf, b2_buf, c_buf,
            st_w1, st_w2, st_w,
            wqT, wkvT, woT, w1N, w2T,
            modT, b1T, b2T, gT_ref, scT, dsc_ref,
            xT, h1T, hnext, kT, vT, stat1, stat2,
            m_state, dm_state,
            qT, qsT, pqT, knat, vnat, vaug, p_ref, sbuf,
            adot, amem, rden, cinv, oT, sA, sB, sC,
            h2T, dffnT, dyT, gactT, duT, dOp, wmemT, dqkvT,
            acc_wqkv, acc_wo, acc_w1T, acc_w2, acc_vec, acc_b1,
            sems):
    def cp(src, dst, k):
        return pltpu.make_async_copy(src, dst, sems.at[k])

    def in_x(s):
        r = pl.ds(_mo(s * L, L), L)
        return cp(x_hbm.at[0, r, :], x_buf.at[r, :], 1 + s)

    in_wmodA = cp(wmod_hbm.at[:, pl.ds(0, 2 * D)], wmod_buf.at[:, pl.ds(0, 2 * D)], 0)
    in_w = [cp(w, wqkv_buf.at[k], 5 + k) for k, w in enumerate((wq_hbm, wk_hbm, wv_hbm))]
    in_wmodB = cp(wmod_hbm.at[:, pl.ds(2 * D, 4 * D)], wmod_buf.at[:, pl.ds(2 * D, 4 * D)], 8)
    in_wo = cp(wo_hbm, wo_buf, 9)
    in_w1 = cp(w1_hbm, w1_buf.at[pl.ds(0, F), :], 10)
    in_w2 = cp(w2_hbm, w2_buf.at[pl.ds(0, F), :], 11)
    in_dy = cp(dy_hbm.at[0], dy_buf, 12)
    in_small = [cp(c_hbm, c_buf, 21), cp(beta_hbm, beta_buf, 22), cp(b1_hbm, b1_buf, 23), cp(b2_hbm, b2_buf, 24)]

    for d in in_small:
        d.start()
    in_x(0).start()
    in_wmodA.start()
    in_w[1].start()
    in_w[2].start()
    in_x(1).start()
    in_w[0].start()
    in_wo.start()
    in_x(2).start()
    in_x(3).start()
    in_wmodB.start()
    in_dy.start()
    in_w1.start()
    in_w2.start()

    dm_state[...] = jnp.zeros(dm_state.shape, f32)
    m_state[0:D, :] = jnp.zeros((D, 128), f32)
    gactT[F // 2:FP // 2, :] = jnp.zeros(((FP - F) // 2, L), u32)
    duT[F // 2:FP // 2, :] = jnp.zeros(((FP - F) // 2, L), u32)
    w1_buf[F:FP, :] = jnp.zeros((FP - F, D), bf16)
    w2_buf[F:FP, :] = jnp.zeros((FP - F, D), bf16)
    dsc_ref[...] = jnp.zeros(dsc_ref.shape, f32)

    for d in in_small:
        d.wait()

    def silu_parts():
        c = c_buf[...].astype(f32)
        sig_c = 1.0 / (1.0 + jnp.exp(-c))
        return c, sig_c

    def gate_row():
        beta = beta_buf[...].astype(f32).reshape(1, H)
        return 1.0 / (1.0 + jnp.exp(-beta))

    def head_onehot():
        return (_iota((D, H), 0) // DH) == _iota((D, H), 1)

    c, sig_c = silu_parts()
    sc = c * sig_c
    sc16 = jnp.broadcast_to(sc, (16, D)).astype(bf16)
    scT[...] = _colrep(sc.astype(bf16).astype(f32))

    def mod_chunks(lo, hi):
        for k in range(lo, hi):
            m = _dot(sc16, wmod_buf[:, k * D:(k + 1) * D], NN)[0:1, :]
            if k in (1, 4):
                m = m + 1.0
            modT[k * D:(k + 1) * D, :] = _colrep(m)

    def P(k, n=L):
        return _rep(modT[k * D:(k + 1) * D, :], n)

    bd80 = (_iota((QR, 128), 0) // DH) == (_iota((QR, 128), 1) // DH)
    lane80 = _iota((QR, 128), 1)
    bd = jnp.logical_and(bd80, lane80 < QR)
    mask2 = jnp.logical_or(bd, jnp.logical_and(
        jnp.logical_and(lane80 >= QR, lane80 < QR + 32),
        ((lane80 - QR) // 8) == (_iota((QR, 128), 0) // DH)))
    ONES_U = jnp.uint32(0x3F803F80)
    zeros24 = jnp.zeros((24, L), u32)
    ones24 = jnp.full((24, L), ONES_U, u32)

    b1row = b1_buf[...].astype(f32).reshape(1, F)
    for k in range(F // 128):
        b1T[k * 128:(k + 1) * 128, :] = _colrep(b1row[:, k * 128:(k + 1) * 128])
    b1T[F - 128:F, :] = _colrep(b1row[:, F - 128:F])
    b2T[...] = _colrep(b2_buf[...].astype(f32).reshape(1, D))
    gcol = jnp.sum(jnp.where(head_onehot(), jnp.broadcast_to(gate_row(), (D, H)), 0.0), axis=1, keepdims=True)
    gT_ref[...] = jnp.broadcast_to(gcol, (D, 128))

    def ln1_tile(s, t):
        lt = slice(t * 128, (t + 1) * 128)
        xt_b = x_buf[pl.ds(_mo(s * L + t * 128, 128), 128), :].T
        xT[pl.ds(_mo(s * (D // 2), 8), D // 2), lt] = _U(xt_b)
        xt = xt_b.astype(f32)
        mu = jnp.mean(xt, axis=0, keepdims=True)
        xc = xt - mu
        var = jnp.mean(xc * xc, axis=0, keepdims=True)
        rstd = jax.lax.rsqrt(var + EPS)
        stat1[pl.ds(_mo(s * 16, 8), 8), lt] = jnp.broadcast_to(mu, (8, 128))
        stat1[pl.ds(_mo(s * 16 + 8, 8), 8), lt] = jnp.broadcast_to(rstd, (8, 128))
        return xc * rstd

    in_x(0).wait()
    for t in range(4):
        sA[:, t * 128:(t + 1) * 128] = ln1_tile(0, t)
    in_wmodA.wait()
    mod_chunks(0, 2)
    hnext[...] = _pack(sA[...] * P(1) + P(0))
    in_w[1].wait()
    wkvT[0:D // 2, :] = _U(wqkv_buf[1].T)
    in_w[2].wait()
    wkvT[D // 2:D, :] = _U(wqkv_buf[2].T)

    def phase0(s, carry):
        @pl.when(s < NSEG - 1)
        def _():
            in_x(s + 1).wait()

        r0 = _mo(s * (D // 2), 8)
        s_next = jnp.minimum(s + 1, NSEG - 1)
        h1T[pl.ds(r0, D // 2), :] = hnext[...]

        def zero_part(k):
            for acc in (acc_wqkv, acc_wo, acc_w1T, acc_w2, acc_vec, acc_b1):
                q = acc.shape[0] // NSEG
                lo, hi = 8 * ((q // 8) * k // 8), 8 * ((q // 8) * (k + 1) // 8)
                acc[pl.ds(_mo(s * q + lo, 8), hi - lo), :] = jnp.zeros((hi - lo, acc.shape[1]), f32)

        for k in range(4):
            hb = _B(h1T[pl.ds(r0, D // 2), :])
            kk = _dot(_B(wkvT[k * 80:(k + 1) * 80, :]), hb, NN)
            kT[pl.ds(r0 + k * 80, 80), :] = _pack(kk)
            pqT[k * 80:(k + 1) * 80, :] = _pack(_phi(kk))
            zero_part(2 * k)
            vv = _dot(_B(wkvT[D // 2 + k * 80:D // 2 + (k + 1) * 80, :]), hb, NN)
            vT[pl.ds(r0 + k * 80, 80), :] = _pack(vv)
            zero_part(2 * k + 1)
            hnext[:, k * 128:(k + 1) * 128] = _pack(ln1_tile(s_next, k) * P(1, 128) + P(0, 128))
            for i in (2 * k, 2 * k + 1):
                pk_u = pqT[i * 40:(i + 1) * 40, :]
                v_aug = jnp.concatenate([vT[pl.ds(r0 + i * 40, 40), :], ones24], axis=0)
                mm = _dot(_B(pk_u), _B(v_aug), NT)
                b0 = _mo(s * D + i * QR, 8)
                m_state[pl.ds(b0 + D, QR), :] = m_state[pl.ds(b0, QR), :] + mm
        return carry

    with _scope("phase0"):
        jax.lax.fori_loop(0, NSEG, phase0, 0)

    in_w[0].wait()
    in_wo.wait()
    in_wmodB.wait()
    wqT[...] = _U(wqkv_buf[0].T)
    woT[...] = _U(wo_buf[...].T)
    mod_chunks(2, 6)
    in_dy.wait()
    in_w1.wait()
    in_w2.wait()

    HL = L // 2

    def out_copy(s, hf):
        r = pl.ds(_mo(s * L + hf * HL, HL), HL)
        return cp(x_buf.at[r, :], out_hbm.at[0, r, :], 25 + 2 * s + hf)

    def dx_copy(s, t):
        r = pl.ds(_mo(s * L + t * 128, 128), 128)
        return cp(dy_buf.at[r, :], dx_hbm.at[0, r, :], 33 + 4 * s + t)

    WCH = D // 4

    def o_w(k, t):
        r = pl.ds(_mo(t * WCH, 16), WCH)
        return cp(st_w.at[k, r, :], (dwq_hbm, dwk_hbm, dwv_hbm)[k].at[r, :], 49 + 4 * k + t)

    o_w1 = cp(st_w1, dw1_hbm, 0)
    o_w2 = cp(st_w2, dw2_hbm, 1)
    o_wo = cp(st_w.at[3], dwo_hbm, 2)
    o_b1 = cp(b1_buf, db1_hbm, 12)
    o_b2 = cp(b2_buf, db2_hbm, 13)
    o_beta = cp(beta_buf, dbeta_hbm, 14)
    o_c = cp(c_buf, dc_hbm, 15)

    def o_mod(k):
        cs = pl.ds(_mo(k * D, 128), D)
        return cp(wmod_buf.at[:, cs], dwmod_hbm.at[:, cs], 6 + k)

    def dmod_chunk(k, c_):
        dm = _rowsum(acc_vec[pl.ds(_mo(k * D, 8), D), :])
        cs = pl.ds(_mo(k * D, 128), D)
        dsc_ref[...] += _dot(jnp.broadcast_to(dm, (16, D)).astype(bf16), wmod_buf[:, cs], NT)
        wmod_buf[:, cs] = (_rep(scT[...], D) * dm).astype(bf16)
        o_mod(k).start()
        return c_

    r40 = _iota((40, 128), 0)
    hmask = [jnp.logical_and(r40 >= 10 * j, r40 < 10 * j + 10) for j in range(4)]

    def segment(it, carry):
        s = NSEG - 1 - it
        r0 = _mo(s * (D // 2), 8)
        tok = pl.ds(_mo(s * L, L), L)
        last = it == NSEG - 1

        hb = _B(h1T[pl.ds(r0, D // 2), :])
        q = _dot(_B(wqT[...]), hb, NN)
        qT[...] = _pack(q)
        qsT[...] = _pack(q * (SCALE * LOG2E))
        pqT[...] = _pack(_phi(q))
        r16 = _iota((16, L), 0)
        for i in range(NQ):
            k_u = kT[pl.ds(r0 + i * 40, 40), :]
            v_u = vT[pl.ds(r0 + i * 40, 40), :]
            knat[i * 256:(i + 1) * 256, :] = _U(_B(jnp.concatenate([k_u, zeros24], axis=0)).T)
            vnat[i * 256:(i + 1) * 256, :] = _U(_B(jnp.concatenate([v_u, ones24], axis=0)).T)
            for j in range(4):
                keep = jnp.logical_and(r16 >= 2 * j, r16 < 2 * j + 10)
                vaug[(4 * i + j) * 16:(4 * i + j + 1) * 16, :] = jnp.where(keep, v_u[8 * j:8 * j + 16], ONES_U)

        def s_weights(i, t):
            qt = qsT[pl.ds(_mo(i * 40, 8), 40), t * 128:(t + 1) * 128]
            wq = jnp.concatenate([jnp.where(hmask[j], qt, jnp.uint32(0)) for j in range(4)], axis=1)
            return _B(jnp.concatenate([wq, zeros24], axis=0))

        def s_tile(i, t, u, mx):
            sc_ = _dot(_B(knat[pl.ds(_mo(i * 256 + u * 64, 8), 64), :]), s_weights(i, t), NN)
            if u == t:
                causal = _iota((128, 128), 0) <= _iota((128, 128), 1)
                sc_ = jnp.concatenate([jnp.where(causal, sc_[:, j * 128:(j + 1) * 128], -1e30)
                                       for j in range(4)], axis=1)
            sbuf[2 * POFF[t] + u * 128:2 * POFF[t] + (u + 1) * 128, :] = sc_
            for k in range(16):
                v = sc_[8 * k:8 * k + 8]
                mx = v if mx is None else jnp.maximum(mx, v)
            if u == t:
                mx = jnp.max(mx, axis=0, keepdims=True)
            return mx

        def p_tile(i, t, u, mx, ws):
            for j in range(4):
                lj = slice(j * 128, (j + 1) * 128)
                sj = sbuf[2 * POFF[t] + u * 128:2 * POFF[t] + (u + 1) * 128, lj]
                p = jnp.exp2(sj - mx[:, lj]).astype(bf16)
                p_ref[pl.ds(_mo(i * 640 + POFF[t] + u * 64, 8), 64), lj] = _U(p)
                va = _B(vaug[pl.ds(_mo((i * 4 + j) * 16, 16), 16), u * 128:(u + 1) * 128])
                w = _dot(va, p, NN)
                ws[j] = w if ws[j] is None else ws[j] + w
            if u == t:
                ls = [1.0 / (ws[j][24:32] if j < 2 else ws[j][0:8]) for j in range(4)]
                linv = _assemble_rows(ls)
                rq = pl.ds(_mo(i * QR, 8), QR)
                adot[rq, t * 128:(t + 1) * 128] = _assemble(ws) * linv
                cinv[rq, t * 128:(t + 1) * 128] = linv * (1.0 - gT_ref[rq, :])

        mx_first = None
        for u in range(4):
            mx_first = s_tile(0, 3, u, mx_first)

        def attn_fwd(i, mx3):
            i_next = jnp.minimum(i + 1, NQ - 1)
            mx = {3: mx3, 2: None, 1: None, 0: None, 4: None}
            ws = {t: [None] * 4 for t in range(4)}
            s_jobs = [(2, 0), (2, 1), (2, 2), (1, 0), (1, 1), (0, 0), (4, 0), (4, 1), (4, 2), (4, 3)]
            p_jobs = [(3, 0), (3, 1), (3, 2), (3, 3), (2, 0), (2, 1), (2, 2), (1, 0), (1, 1), (0, 0)]
            for (st, su), (pt, pu) in zip(s_jobs, p_jobs):
                if st == 4:
                    mx[4] = s_tile(i_next, 3, su, mx[4])
                else:
                    mx[st] = s_tile(i, st, su, mx[st])
                p_tile(i, pt, pu, mx[pt], ws[pt])
            rq = pl.ds(_mo(i * QR, 8), QR)
            mm = m_state[pl.ds(_mo(s * D + i * QR, 8), QR), :]
            mt = jnp.concatenate([mm, jnp.zeros((48, 128), f32)], axis=0).T
            zrep = jnp.concatenate([mt[QR:QR + 8]] * 10, axis=0)
            lhs = jnp.concatenate([jnp.where(bd, mt[0:QR], 0.0), jnp.where(bd, zrep, 0.0)], axis=0).astype(bf16)
            pq_w = _B(jnp.concatenate([pqT[pl.ds(_mo(i * 40, 8), 40), :], zeros24], axis=0))
            nd = _dot(lhs, pq_w, NN)
            rd = 1.0 / (nd[QR:] + 1e-6)
            am = nd[0:QR] * rd
            amem[rq, :] = am
            g = _rep(gT_ref[rq, :])
            rden[rq, :] = g * rd
            o = g * am + (1.0 - g) * adot[rq, :]
            oT[pl.ds(_mo(i * 40, 8), 40), :] = _pack(o)
            return mx[4]

        with _scope("attn_fwd"):
            jax.lax.fori_loop(0, NQ, attn_fwd, mx_first)

        dyT[...] = _U(dy_buf[tok, :].T)
        dffn = _B(dyT[...]).astype(f32) * P(5)
        dffnT[...] = _pack(dffn)
        acc_vec[6 * D:7 * D, :] += _fold(dffn)
        attn = _dot(_B(woT[...]), _B(oT[...]), NN)
        sA[...] = attn
        x2 = _B(xT[pl.ds(r0, D // 2), :]).astype(f32) + P(2) * attn
        sB[...] = x2
        mu2 = jnp.mean(x2, axis=0, keepdims=True)
        xc2 = x2 - mu2
        var2 = jnp.mean(xc2 * xc2, axis=0, keepdims=True)
        rstd2 = jax.lax.rsqrt(var2 + EPS)
        xh2 = xc2 * rstd2
        sC[...] = xh2
        h2T[...] = _pack(xh2 * P(4) + P(3))
        stat2[...] = jnp.broadcast_to(rstd2, (8, L))

        def ffn_chunk(ci, c_):
            rp = pl.ds(_mo(ci * (FCH // 2), 8), FCH // 2)
            rf = pl.ds(_mo(ci * FCH, 16), FCH)
            h2b = _B(h2T[...])
            dfb = _B(dffnT[...])
            u = _dot(w1_buf[rf, :], h2b, NN) + _rep(b1T[rf, :])
            dg = _dot(w2_buf[rf, :], dfb, NN)
            u2 = u * u
            th = jnp.tanh(u * (GELU_C1 + GELU_C2 * u2))
            hp = 0.5 * th + 0.5
            gactT[rp, :] = _pack(u * hp)
            gp = hp + (0.5 * u) * (1.0 - th * th) * (GELU_C1 + (3.0 * GELU_C2) * u2)
            du = dg * gp
            duT[rp, :] = _pack(du)
            acc_b1[rf, :] += _fold(du)
            a2 = acc_w2[rf, :] + _dot(_B(gactT[rp, :]), dfb, NT)
            acc_w2[rf, :] = a2
            st_w2[rf, :] = a2.astype(bf16)
            a1 = acc_w1T[rf, :] + _dot(_B(duT[rp, :]), h2b, NT)
            acc_w1T[rf, :] = a1
            st_w1[rf, :] = a1.astype(bf16)
            for blk in (ci, ci + NFC, jnp.minimum(ci + 2 * NFC, FP // 128 - 1)):
                rb = pl.ds(_mo(blk * 128, 128), 128)
                w1N[:, rb] = _U(w1_buf[rb, :].T)
                w2T[:, rb] = _U(w2_buf[rb, :].T)
            return c_

        with _scope("ffn_chunk"):
            jax.lax.fori_loop(0, NFC, ffn_chunk, 0)

        @pl.when(last)
        def _():
            o_w1.start()
            o_w2.start()

        def post_ffn(hf, c_):
            hl = pl.ds(_mo(hf * HL, HL), HL)
            rows = pl.ds(_mo(s * L + hf * HL, HL), HL)
            dh2 = _dot(_B(w1N[...]), _B(duT[:, hl]), NN)
            dyt = _B(dyT[:, hl]).astype(f32)
            xh2 = sC[:, hl]
            acc_vec[3 * D:4 * D, :] += _fold(dh2)
            acc_vec[4 * D:5 * D, :] += _fold(dh2 * xh2)
            dxh = dh2 * P(4, HL)
            m1 = jnp.mean(dxh, axis=0, keepdims=True)
            m2 = jnp.mean(dxh * xh2, axis=0, keepdims=True)
            dx2 = dyt + stat2[0:1, hl] * (dxh - m1 - xh2 * m2)
            sC[:, hl] = dx2
            acc_vec[2 * D:3 * D, :] += _fold(dx2 * sA[:, hl])
            dffnT[:, hl] = _pack(dx2 * P(2, HL))
            ffn = _dot(_B(w2T[...]), _B(gactT[:, hl]), NN) + _rep(b2T[...], HL)
            acc_vec[5 * D:6 * D, :] += _fold(_B(dyT[:, hl]).astype(f32) * ffn)
            outT = sB[:, hl] + P(5, HL) * ffn
            x_buf[rows, :] = outT.astype(bf16).T
            dab = _B(dffnT[:, hl])
            do_all = _dot(wo_buf[...], dab, NN)
            for i in range(NQ):
                rq = slice(i * QR, (i + 1) * QR)
                do = do_all[rq]
                ad = adot[rq, hl]
                am = amem[rq, hl]
                acc_vec[7 * D + i * QR:7 * D + (i + 1) * QR, :] += _fold(do * (am - ad))
                dOp[i * 72:i * 72 + 40, hl] = _pack(do * cinv[rq, hl])
                parts = _head_partials(_B(dOp[i * 72:i * 72 + 40, hl]).astype(f32) * ad)
                for j in range(4):
                    hi = (-parts[j]).astype(bf16).astype(f32)
                    lo = -parts[j] - hi
                    dOp[i * 72 + 40 + 8 * j:i * 72 + 48 + 8 * j, hl] = _pack(jnp.concatenate([hi, lo], axis=0))
                dnum = do * rden[rq, hl]
                tp = _head_partials(dnum * am)
                wmemT[i * 56:(i + 1) * 56, hl] = _pack(jnp.concatenate([dnum] + [-x for x in tp], axis=0))
            ao = acc_wo[...] + _dot(_B(oT[:, hl]), dab, NT)
            acc_wo[...] = ao
            st_w[3] = ao.astype(bf16)
            out_copy(s, hf).start()
            return c_

        with _scope("post_ffn"):
            jax.lax.fori_loop(0, 2, post_ffn, 0)

        @pl.when(last)
        def _():
            o_wo.start()
            jax.lax.fori_loop(2, 6, dmod_chunk, 0)
            b2_buf[...] = _rowsum(acc_vec[6 * D:7 * D, :]).reshape(D).astype(bf16)
            o_b2.start()
            parts = [_rowsum(acc_b1[k * 128:(k + 1) * 128, :]) for k in range(F // 128)]
            parts.append(_rowsum(acc_b1[F - 128:F, :])[:, 64:128])
            b1_buf[...] = jnp.concatenate(parts, axis=1).reshape(F).astype(bf16)
            o_b1.start()

        def attn_bwd(i, c_):
            rq = pl.ds(_mo(i * QR, 8), QR)
            rp = pl.ds(_mo(i * 40, 8), 40)
            d0 = _mo(i * 72, 8)
            dq = [[None] * 4 for _ in range(4)]
            dk = [[None] * 4 for _ in range(4)]
            dv = [[None] * 4 for _ in range(4)]
            mem = {}

            def wmem():
                return _B(jnp.concatenate([wmemT[pl.ds(_mo(i * 56, 8), 56), :], jnp.zeros((8, L), u32)], axis=0))

            def mem_dq():
                mm = m_state[pl.ds(_mo(s * D + i * QR, 8), QR), :]
                dpq = _dot(jnp.where(mask2, mm, 0.0).astype(bf16), wmem(), NN)
                qq = _B(qT[rp, :]).astype(f32)
                mem['q'] = dpq * jnp.where(qq > 0, 1.0, _B(pqT[rp, :]).astype(f32))

            def mem_dkv():
                kk = _B(kT[pl.ds(r0 + i * 40, 40), :]).astype(f32)
                pk = _phi(kk)
                pk_w = jnp.concatenate([pk, jnp.zeros((48, L), f32)], axis=0).astype(bf16)
                v_aug = _B(jnp.concatenate([vT[pl.ds(r0 + i * 40, 40), :], ones24], axis=0))
                dms = dm_state[rq, :]
                dpk = _dot(jnp.where(mask2, dms, 0.0).astype(bf16), v_aug, NN)
                dmt = jnp.concatenate([jnp.where(bd, dms, 0.0), jnp.zeros((48, 128), f32)], axis=0).T
                mem['v'] = _dot(dmt[0:QR].astype(bf16), pk_w, NN)
                mem['k'] = dpk * jnp.where(kk > 0, 1.0, pk)

            def mem_update():
                dm_state[rq, :] += _dot(_B(pqT[rp, :]), wmem(), NT)

            def dp_tile(t, u):
                lt = slice(t * 128, (t + 1) * 128)
                dt = dOp[pl.ds(d0, 40), lt]
                wd = jnp.concatenate(
                    [jnp.concatenate([jnp.where(hmask[j], dt, jnp.uint32(0)), dOp[pl.ds(d0 + 40 + 8 * j, 8), lt],
                                      jnp.zeros((16, 128), u32)], axis=0) for j in range(4)], axis=1)
                dp = _dot(_B(vnat[pl.ds(_mo(i * 256 + u * 64, 8), 64), :]), _B(wd), NN)
                res = []
                for j in range(4):
                    p = _B(p_ref[pl.ds(_mo(i * 640 + POFF[t] + u * 64, 8), 64), j * 128:(j + 1) * 128])
                    res.append((dp[:, j * 128:(j + 1) * 128] * p.astype(f32)).astype(bf16))
                return res

            def thin_tile(t, u, ds):
                lt = slice(t * 128, (t + 1) * 128)
                for j in range(4):
                    p = _B(p_ref[pl.ds(_mo(i * 640 + POFF[t] + u * 64, 8), 64), j * 128:(j + 1) * 128])
                    kw = _B(kT[pl.ds(r0 + i * 40 + 8 * j, 16), u * 128:(u + 1) * 128])
                    qw = _B(qT[pl.ds(_mo(i * 40 + 8 * j, 8), 16), lt])
                    dw = _B(dOp[pl.ds(d0 + 8 * j, 16), lt])
                    b = _dot(dw, p, NT)
                    a = _dot(qw, ds[j], NT)
                    e = _dot(kw, ds[j], NN)
                    dq[j][t] = e if dq[j][t] is None else dq[j][t] + e
                    dk[j][u] = a if dk[j][u] is None else dk[j][u] + a
                    dv[j][u] = b if dv[j][u] is None else dv[j][u] + b
                if u == t:
                    col = lambda w: _assemble([w[j][t] for j in range(4)])
                    dqkvT[rp, lt] = _pack(col(dq) * SCALE + mem['q'][:, lt])
                    dqkvT[pl.ds(_mo(D // 2 + i * 40, 8), 40), lt] = _pack(col(dk) * SCALE + mem['k'][:, lt])
                    dqkvT[pl.ds(_mo(D + i * 40, 8), 40), lt] = _pack(col(dv) + mem['v'][:, lt])

            jobs = [(t, u) for t in (3, 2, 1, 0) for u in range(t + 1)]
            extra = {0: mem_dq, 1: mem_dkv, 9: mem_update}
            ds = dp_tile(*jobs[0])
            for n_, job in enumerate(jobs):
                ds_next = dp_tile(*jobs[n_ + 1]) if n_ + 1 < len(jobs) else None
                if n_ in extra:
                    extra[n_]()
                thin_tile(job[0], job[1], ds)
                ds = ds_next
            return c_

        with _scope("attn_bwd"):
            jax.lax.fori_loop(0, NQ, attn_bwd, 0)

        def qkv_bwd(t, c_):
            lt = pl.ds(_mo(t * 128, 128), 128)
            rows = pl.ds(_mo(s * L + t * 128, 128), 128)
            dh1 = _dot(wqkv_buf[0], _B(dqkvT[0:D // 2, lt]), NN)
            dh1 = dh1 + _dot(wqkv_buf[1], _B(dqkvT[D // 2:D, lt]), NN)
            dh1 = dh1 + _dot(wqkv_buf[2], _B(dqkvT[D:3 * D // 2, lt]), NN)
            mu = stat1[pl.ds(_mo(s * 16, 8), 1), lt]
            rstd = stat1[pl.ds(_mo(s * 16 + 8, 8), 1), lt]
            xh1 = (_B(xT[pl.ds(r0, D // 2), lt]).astype(f32) - mu) * rstd
            acc_vec[0:D, :] += dh1
            acc_vec[D:2 * D, :] += dh1 * xh1
            dxh = dh1 * P(1, 128)
            m1 = jnp.mean(dxh, axis=0, keepdims=True)
            m2 = jnp.mean(dxh * xh1, axis=0, keepdims=True)
            dx = sC[:, lt] + rstd * (dxh - m1 - xh1 * m2)
            dy_buf[rows, :] = dx.astype(bf16).T
            ra = pl.ds(_mo(t * WCH, 16), WCH)
            aw = acc_wqkv[ra, :] + _dot(_B(h1T[pl.ds(r0 + t * (WCH // 2), WCH // 2), :]), _B(dqkvT[...]), NT)
            acc_wqkv[ra, :] = aw
            for k in range(3):
                st_w[k, ra, :] = aw[:, k * D:(k + 1) * D].astype(bf16)
            dx_copy(s, t).start()

            @pl.when(last)
            def _():
                for k in range(3):
                    o_w(k, t).start()
            return c_

        with _scope("qkv_bwd"):
            jax.lax.fori_loop(0, 4, qkv_bwd, 0)

        @pl.when(last)
        def _():
            jax.lax.fori_loop(0, 2, dmod_chunk, 0)
            c_, sig = silu_parts()
            c_buf[...] = (dsc_ref[0:1, :] * (sig * (1.0 + c_ * (1.0 - sig)))).astype(bf16)
            o_c.start()
            gate = gate_row()
            dgc = jnp.sum(acc_vec[7 * D:8 * D, :], axis=1, keepdims=True)
            dgate = jnp.sum(jnp.where(head_onehot(), jnp.broadcast_to(dgc, (D, H)), 0.0), axis=0, keepdims=True)
            beta_buf[...] = (dgate * gate * (1.0 - gate)).reshape(H).astype(bf16)
            o_beta.start()

        return carry

    with _scope("segment"):
        jax.lax.fori_loop(0, NSEG, segment, 0)

    for s in range(NSEG):
        for hf in range(2):
            out_copy(s, hf).wait()
        for t in range(4):
            dx_copy(s, t).wait()
    for d in [o_w2, o_w1, o_wo, o_b1, o_b2, o_beta, o_c] + [o_mod(k) for k in range(6)] + [
            o_w(k, t) for k in range(3) for t in range(4)]:
        d.wait()


@jax.jit
def pallas_adaLN_cond__memory_aug_infini_attn__dense_activation_gelu__prompt_kernel(
    A_x: jax.Array,
    A_wq: jax.Array,
    A_wk: jax.Array,
    A_wv: jax.Array,
    A_wo: jax.Array,
    A_beta: jax.Array,
    B_x: jax.Array,
    B_w1: jax.Array,
    B_b1: jax.Array,
    B_w2: jax.Array,
    B_b2: jax.Array,
    c: jax.Array,
    w_mod: jax.Array,
    grad_out: jax.Array,
):
    del B_x
    hbm = pl.BlockSpec(memory_space=pltpu.HBM)
    sds = jax.ShapeDtypeStruct
    V = pltpu.VMEM
    scratch = [
        V((S, D), bf16), V((S, D), bf16), V((3, D, D), bf16), V((D, D), bf16), V((FP, D), bf16),
        V((FP, D), bf16), V((D, 6 * D), bf16),
        V((H,), bf16), V((F,), bf16), V((D,), bf16), V((1, D), bf16),
        V((F, D), bf16), V((F, D), bf16), V((4, D, D), bf16),
        V((D // 2, D), u32), V((D, D), u32), V((D // 2, D), u32), V((D // 2, FP), u32), V((D // 2, FP), u32),
        V((6 * D, 128), f32), V((F, 128), f32), V((D, 128), f32), V((D, 128), f32), V((D, 128), f32),
        V((16, D), f32),
        V((NSEG * D // 2, L), u32), V((NSEG * D // 2, L), u32), V((D // 2, L), u32), V((NSEG * D // 2, L), u32),
        V((NSEG * D // 2, L), u32), V((NSEG * 16, L), f32), V((8, L), f32),
        V(((NSEG + 1) * D, 128), f32), V((D, 128), f32),
        V((D // 2, L), u32), V((D // 2, L), u32), V((D // 2, L), u32),
        V((NQ * 256, 128), u32), V((NQ * 256, 128), u32), V((H * 16, L), u32), V((NQ * 640, L), u32), V((1280, L), f32),
        V((D, L), f32), V((D, L), f32), V((D, L), f32), V((D, L), f32), V((D // 2, L), u32),
        V((D, L), f32), V((D, L), f32), V((D, L), f32),
        V((D // 2, L), u32), V((D // 2, L), u32), V((D // 2, L), u32), V((FP // 2, L), u32), V((FP // 2, L), u32),
        V((NQ * 72, L), u32), V((NQ * 56, L), u32), V((3 * D // 2, L), u32),
        V((D, 3 * D), f32), V((D, D), f32), V((F, D), f32), V((F, D), f32), V((8 * D, 128), f32),
        V((F, 128), f32),
        pltpu.SemaphoreType.DMA((61,)),
    ]
    outs = pl.pallas_call(
        _kernel,
        in_specs=[hbm] * 13,
        out_specs=[hbm] * 13,
        out_shape=[
            sds((1, S, D), bf16), sds((1, S, D), bf16), sds((D, D), bf16), sds((D, D), bf16),
            sds((D, D), bf16), sds((D, D), bf16), sds((H,), bf16), sds((F, D), bf16), sds((F,), bf16),
            sds((F, D), bf16), sds((D,), bf16), sds((1, D), bf16), sds((D, 6 * D), bf16),
        ],
        scratch_shapes=scratch,
        compiler_params=pltpu.CompilerParams(vmem_limit_bytes=124 * 1024 * 1024),
    )(A_x, A_wq, A_wk, A_wv, A_wo, A_beta, B_w1.T, B_b1, B_w2, B_b2, c, w_mod, grad_out)
    out, dx, dwq, dwk, dwv, dwo, dbeta, dw1, db1, dw2, db2, dc, dwmod = outs
    return (out, dx, dwq, dwk, dwv, dwo, dbeta, dw1.T, db1, dw2, db2, dc, dwmod)
```

```python
import contextlib
import math

import jax
import jax.numpy as jnp
import jax.experimental.pallas as pl
import jax.experimental.pallas.tpu as pltpu

bf16 = jnp.bfloat16
f32 = jnp.float32
u32 = jnp.uint32

S, D, H, DH, NSEG, L, F = 2048, 640, 32, 20, 4, 512, 1728
FP = 1792
NQ = 8
QR = 80
FCH = 288
NFC = F // FCH
SCALE = DH ** -0.5
LOG2E = math.log2(math.e)
GELU_C1 = math.sqrt(2.0 / math.pi)
GELU_C2 = GELU_C1 * 0.044715
EPS = 1e-5
POFF = (0, 64, 192, 384)

_PROFILE = False
QP = 4
RSP = 3
ML = 1
UF, UB, UC = 2, 4, 2
MPOS = 2
TIE0 = 0
LAGT = 4
RC = 16
RC0 = 32
_FSPLIT = 640
_DWO_POS = (2, 4, 6, 7, 8)


def _scope(name):
    return jax.named_scope(name) if _PROFILE else contextlib.nullcontext()


NN = (((1,), (0,)), ((), ()))
NT = (((1,), (1,)), ((), ()))


def _dot(a, b, dims):
    return jax.lax.dot_general(a, b, dims, preferred_element_type=f32)


def _B(x):
    return pltpu.bitcast(x, bf16)


def _U(x):
    return pltpu.bitcast(x, u32)


def _pack(x):
    return _U(x.astype(bf16))


def _iota(shape, dim):
    return jax.lax.broadcasted_iota(jnp.int32, shape, dim)


def _rep(p, n=L):
    return jnp.concatenate([p] * (n // 128), axis=1)


def _fold(x):
    acc = x[:, 0:128]
    for t in range(1, x.shape[1] // 128):
        acc = acc + x[:, t * 128:(t + 1) * 128]
    return acc


def _vsum(x, acc=None):
    for k in range(x.shape[0] // 8):
        v = x[8 * k:8 * k + 8]
        acc = v if acc is None else acc + v
    return acc


class _Chain:
    def __init__(self, idx, lag=1):
        self.lag = lag
        self.true = None if idx is None else _iota((8, 128), 0) >= jnp.minimum(idx, 0)
        self.done = []

    def tie(self, x, rows):
        if self.true is not None and len(self.done) >= self.lag:
            x = jnp.where(self.true, x, self.done[-self.lag])
        return jnp.concatenate([x] * (rows // 8), axis=0)

    def push(self, y):
        self.done.append(y[y.shape[0] - 8:, 0:128])


def _loop(n, body, init, unroll):
    def wide(i, c):
        for k in range(unroll):
            c = body(i * unroll + k, c)
        return c
    return jax.lax.fori_loop(0, n // unroll, wide, init)


def _colrep(row):
    return jnp.broadcast_to(row, (128, row.shape[1])).T


def _rowsum(acc):
    return jnp.sum(acc.T, axis=0, keepdims=True)


def _phi(x):
    return jnp.where(x > 0, x + 1.0, jnp.exp(x))


def _mo(x, m):
    return pl.multiple_of(x, m)


def _swap(x):
    return pltpu.roll(x, 64, 1)


def _lt(t):
    return slice(t * 128, (t + 1) * 128) if isinstance(t, int) else pl.ds(_mo(t * 128, 128), 128)


def _assemble(w):
    lo = _iota((8, w[0].shape[1]), 0) < 4
    return jnp.concatenate([
        w[0][0:16], jnp.where(lo, w[0][16:24], w[1][0:8]), w[1][8:24],
        w[2][8:24], jnp.where(lo, w[2][24:32], w[3][8:16]), w[3][16:32]], axis=0)


def _assemble_rows(r):
    lo = _iota(r[0].shape, 0) < 4
    return jnp.concatenate([
        r[0], r[0], jnp.where(lo, r[0], r[1]), r[1], r[1],
        r[2], r[2], jnp.where(lo, r[2], r[3]), r[3], r[3]], axis=0)


def _head_partials(x):
    lo = _iota((8, x.shape[1]), 0) < 4
    v = [x[8 * k:8 * k + 8] for k in range(10)]
    return [v[0] + v[1] + jnp.where(lo, v[2], 0.0),
            jnp.where(lo, 0.0, v[2]) + v[3] + v[4],
            v[5] + v[6] + jnp.where(lo, v[7], 0.0),
            jnp.where(lo, 0.0, v[7]) + v[8] + v[9]]


def _kernel(x_hbm, wq_hbm, wk_hbm, wv_hbm, wo_hbm, beta_hbm, w1_hbm, b1_hbm, w2_hbm, b2_hbm,
            c_hbm, wmod_hbm, dy_hbm,
            out_hbm, dx_hbm, dwq_hbm, dwk_hbm, dwv_hbm, dwo_hbm, dbeta_hbm, dw1_hbm, db1_hbm,
            dw2_hbm, db2_hbm, dc_hbm, dwmod_hbm,
            x_buf, dy_buf, wqkv_buf, w1_buf, w2_buf, wmod_buf,
            beta_buf, b1_buf, b2_buf, c_buf,
            st_w1, st_w2, st_w,
            wqoT, wkvT, w1N, w2T,
            modT, b1T, b2T, gT_ref, scT, dsc_ref, dscT, st_mod,
            xT, hnext, stat1, h1T, kT, vT, stat2,
            m_state, dm_state,
            qT, qsT, pqT, knat, vnat, vaug, p_ref, sbuf,
            adot, amem, rden, cinv, oT, sA, sB, sC, sD,
            h2T, dffnT, dyT, gactT, duT, dOp, wmemT, dqkvT,
            acc_wqkv, acc_wo, acc_w1T, acc_w2, acc_vec, rowbuf,
            sems):
    def cp(src, dst, k):
        return pltpu.make_async_copy(src, dst, sems.at[k])

    def in_x(s):
        r = pl.ds(_mo(s * L, L), L)
        return cp(x_hbm.at[0, r, :], x_buf.at[r, :], 1 + s)

    in_wmodA = cp(wmod_hbm.at[:, pl.ds(0, 2 * D)], wmod_buf.at[:, pl.ds(0, 2 * D)], 0)
    in_w = {0: cp(wq_hbm, wqkv_buf.at[0], 5), 2: cp(wv_hbm, wqkv_buf.at[2], 7), 3: cp(wo_hbm, wqkv_buf.at[3], 9)}
    in_wmodB = cp(wmod_hbm.at[:, pl.ds(2 * D, 4 * D)], wmod_buf.at[:, pl.ds(2 * D, 4 * D)], 8)
    in_w1 = cp(w1_hbm, w1_buf.at[pl.ds(0, F), :], 10)
    in_w2 = cp(w2_hbm, w2_buf.at[pl.ds(0, F), :], 11)
    in_dy = cp(dy_hbm.at[0], dy_buf, 12)
    in_small = [cp(c_hbm, c_buf, 21), cp(beta_hbm, beta_buf, 22), cp(b1_hbm, b1_buf, 23), cp(b2_hbm, b2_buf, 24)]

    for d in in_small:
        d.start()
    in_wk = [cp(wk_hbm.at[pl.ds(lo, n), :], wqkv_buf.at[1, pl.ds(lo, n), :], k)
             for lo, n, k in ((0, 512, 6), (512, 128, 16))]
    for d in [in_x(0), in_w[2], in_wmodA, in_wk[0], in_wk[1], in_x(1), in_w[0], in_x(2), in_w[3],
              in_x(3), in_wmodB, in_dy, in_w1, in_w2]:
        d.start()

    dm_state[...] = jnp.zeros(dm_state.shape, f32)
    m_state[0:D, :] = jnp.zeros((D, 128), f32)
    gactT[F // 2:FP // 2, :] = jnp.zeros(((FP - F) // 2, L), u32)
    duT[F // 2:FP // 2, :] = jnp.zeros(((FP - F) // 2, L), u32)
    w1_buf[F:FP, :] = jnp.zeros((FP - F, D), bf16)
    w2_buf[F:FP, :] = jnp.zeros((FP - F, D), bf16)
    dsc_ref[...] = jnp.zeros(dsc_ref.shape, f32)
    dscT[...] = jnp.zeros(dscT.shape, f32)

    def zero_acc(k, c_):
        acc_vec[pl.ds(_mo(k * D, 8), D), :] = jnp.zeros((D, 128), f32)
        return c_

    jax.lax.fori_loop(0, 11, zero_acc, 0)

    for d in in_small:
        d.wait()

    def silu_parts():
        c = c_buf[...].astype(f32)
        sig_c = 1.0 / (1.0 + jnp.exp(-c))
        return c, sig_c

    def gate_row():
        beta = beta_buf[...].astype(f32).reshape(1, H)
        return 1.0 / (1.0 + jnp.exp(-beta))

    def head_onehot():
        return (_iota((D, H), 0) // DH) == _iota((D, H), 1)

    c, sig_c = silu_parts()
    sc = c * sig_c
    sc16 = jnp.broadcast_to(sc, (16, D)).astype(bf16)
    scT[...] = _colrep(sc.astype(bf16).astype(f32))

    def mod_chunks(lo, hi):
        for k in range(lo, hi):
            m = _dot(sc16, wmod_buf[:, k * D:(k + 1) * D], NN)[0:1, :]
            if k in (1, 4):
                m = m + 1.0
            modT[k * D:(k + 1) * D, :] = _colrep(m)

    def P(k, n=L):
        return _rep(modT[k * D:(k + 1) * D, :], n)

    bd80 = (_iota((QR, 128), 0) // DH) == (_iota((QR, 128), 1) // DH)
    lane80 = _iota((QR, 128), 1)
    bd = jnp.logical_and(bd80, lane80 < QR)
    mask2 = jnp.logical_or(bd, jnp.logical_and(
        jnp.logical_and(lane80 >= QR, lane80 < QR + 32),
        ((lane80 - QR) // 8) == (_iota((QR, 128), 0) // DH)))
    ONES_U = jnp.uint32(0x3F803F80)
    zeros24 = jnp.zeros((24, L), u32)
    ones24 = jnp.full((24, L), ONES_U, u32)

    b1row = b1_buf[...].astype(f32).reshape(1, F)
    for k in range(F // 128):
        b1T[k * 128:(k + 1) * 128, :] = _colrep(b1row[:, k * 128:(k + 1) * 128])
    b1T[F - 128:F, :] = _colrep(b1row[:, F - 128:F])
    b2T[...] = _colrep(b2_buf[...].astype(f32).reshape(1, D))
    gcol = jnp.sum(jnp.where(head_onehot(), jnp.broadcast_to(gate_row(), (D, H)), 0.0), axis=1, keepdims=True)
    gT_ref[...] = jnp.broadcast_to(gcol, (D, 128))

    def x_tile(s, t):
        xt_b = x_buf[pl.ds(_mo(s * L + t * 128, 128), 128), :].T
        xT[pl.ds(_mo(s * (D // 2), 8), D // 2), _lt(t)] = _U(xt_b)

    def ln1_stats(s, t, chain):
        lt = _lt(t)
        ld = lambda r: _B(xT[pl.ds(_mo(s * (D // 2) + r // 2, 8), RC0 // 2), lt]).astype(f32)
        acc = chain.tie(jnp.zeros((8, 128), f32), 8)
        for r in range(0, D, RC0):
            acc = _vsum(ld(r), acc)
        mu = jnp.sum(acc, axis=0, keepdims=True) * (1.0 / D)
        stat1[pl.ds(_mo(s * 16, 8), 8), lt] = jnp.broadcast_to(mu, (8, 128))
        acc = None
        for r in range(0, D, RC0):
            xc = ld(r) - mu
            acc = _vsum(xc * xc, acc)
        rstd = jax.lax.rsqrt(jnp.sum(acc, axis=0, keepdims=True) * (1.0 / D) + EPS)
        stat1[pl.ds(_mo(s * 16 + 8, 8), 8), lt] = jnp.broadcast_to(rstd, (8, 128))
        return jnp.broadcast_to(mu, (8, 128)), rstd

    def ln1_apply(s, t, mu, rstd, chain):
        lt = _lt(t)
        for r in range(0, D, RC0):
            x = _B(xT[pl.ds(_mo(s * (D // 2) + r // 2, 8), RC0 // 2), lt]).astype(f32)
            h = (x - chain.tie(mu, RC0)) * rstd * modT[D + r:D + r + RC0, :] + modT[r:r + RC0, :]
            h = _pack(h)
            chain.push(pltpu.bitcast(h, f32))
            hnext[r // 2:(r + RC0) // 2, lt] = h

    in_x(0).wait()

    def ln0_stats(t, c_):
        x_tile(0, t)
        ln1_stats(0, t, _Chain(None))
        return c_

    def ln0_apply(t, c_):
        ln1_apply(0, t, stat1[0:8, _lt(t)], stat1[8:9, _lt(t)], _Chain(None))
        return c_

    def w_tr(k, r):
        def f(t, c_):
            wkvT[r:r + D // 2, _lt(t)] = _U(wqkv_buf[k, _lt(t), :].T)
            return c_
        return f

    jax.lax.fori_loop(0, 4, ln0_stats, 0)
    in_w[2].wait()
    jax.lax.fori_loop(0, 5, w_tr(2, D // 2), 0)
    in_wmodA.wait()
    mod_chunks(0, 2)
    jax.lax.fori_loop(0, 4, ln0_apply, 0)
    in_wk[0].wait()
    jax.lax.fori_loop(0, 4, w_tr(1, 0), 0)
    in_wk[1].wait()
    w_tr(1, 0)(4, 0)

    def phase0(s, carry):
        @pl.when(s < NSEG - 1)
        def _():
            in_x(s + 1).wait()

        @pl.when(s == 2)
        def _():
            in_w[0].wait()
            in_w[3].wait()
            in_wmodB.wait()

        r0 = _mo(s * (D // 2), 8)
        s_next = jnp.minimum(s + 1, NSEG - 1)
        h1T[pl.ds(r0, D // 2), :] = hnext[...]
        chain = _Chain(s)

        for k in range(4):
            x_tile(s_next, k)
        for k in range(4):
            vv = _dot(_B(wkvT[D // 2 + k * 80:D // 2 + (k + 1) * 80, :]), _B(h1T[pl.ds(r0, D // 2), :]), NN)
            vT[pl.ds(r0 + k * 80, 80), :] = _pack(vv)
            mu, rstd = ln1_stats(s_next, k, chain)
            ln1_apply(s_next, k, mu, rstd, chain)
            kk = _dot(_B(wkvT[k * 80:(k + 1) * 80, :]), _B(h1T[pl.ds(r0, D // 2), :]), NN)
            kT[pl.ds(r0 + k * 80, 80), :] = _pack(kk)
            pqT[0:80, :] = _pack(_phi(kk))
            for i in (2 * k, 2 * k + 1):
                pk_u = pqT[(i % 2) * 40:(i % 2 + 1) * 40, :]
                v_aug = jnp.concatenate([vT[pl.ds(r0 + i * 40, 40), :], ones24], axis=0)
                mm = _dot(_B(pk_u), _B(v_aug), NT)
                b0 = _mo(s * D + i * QR, 8)
                m_state[pl.ds(b0 + D, QR), :] = m_state[pl.ds(b0, QR), :] + mm
        late = s >= 2
        chain2 = _Chain(s, ML)
        src = jnp.where(late, 3 * (s - 2), 1)
        wqoT[pl.ds(_mo((s % 2) * (D // 2), 8), D // 2), :] = _U(wqkv_buf[src].T)
        for j in range(2):
            k = jnp.where(late, 2 * s - 2, 0) + j
            acc = [None] * 5
            for r in range(0, D, RC0):
                w = wmod_buf[r:r + RC0, pl.ds(_mo(k * D, 128), D)].astype(f32)
                for n in range(5):
                    sc_r = jnp.concatenate([chain2.tie(scT[q:q + 8, :], 8) for q in range(r, r + RC0, 8)], axis=0)
                    acc[n] = _vsum(w[:, n * 128:(n + 1) * 128] * sc_r, acc[n])
                    chain2.push(acc[n])
            m = jnp.sum(jnp.concatenate(acc, axis=1), axis=0, keepdims=True) + jnp.where(k == 4, 1.0, 0.0)
            modT[pl.ds(_mo(jnp.where(late, k, 6 + j) * D, 8), D), :] = _colrep(m)
        return carry

    with _scope("phase0"):
        jax.lax.fori_loop(0, NSEG, phase0, 0)

    in_dy.wait()
    in_w1.wait()
    in_w2.wait()

    HL = L // 2

    def out_copy(s, hf):
        r = pl.ds(_mo(s * L + hf * HL, HL), HL)
        return cp(x_buf.at[r, :], out_hbm.at[0, r, :], 25 + 2 * s + hf)

    def dx_copy(s, hf):
        r = pl.ds(_mo(s * L + hf * HL, HL), HL)
        return cp(dy_buf.at[r, :], dx_hbm.at[0, r, :], 33 + 2 * s + hf)

    WCH = D // 4

    def o_w(k, t):
        r = pl.ds(_mo(t * WCH, 16), WCH)
        return cp(st_w.at[k, r, :], (dwq_hbm, dwk_hbm, dwv_hbm)[k].at[r, :], 49 + 4 * k + t)

    o_w1 = cp(st_w1, dw1_hbm, 0)
    o_w2 = cp(st_w2, dw2_hbm, 1)
    o_wo = cp(st_w.at[3], dwo_hbm, 2)
    o_b1 = cp(b1_buf, db1_hbm, 12)
    o_b2 = cp(b2_buf, db2_hbm, 13)
    o_beta = cp(beta_buf, dbeta_hbm, 14)
    o_c = cp(c_buf, dc_hbm, 15)

    def o_mod(k):
        cs = pl.ds(_mo(k * 2 * D, 128), 2 * D)
        return cp(st_mod.at[:, cs], dwmod_hbm.at[:, cs], 6 + k)

    def o_mod01(t):
        r = pl.ds(_mo(t * WCH, 16), WCH)
        return cp(st_mod.at[r, pl.ds(0, 2 * D)], dwmod_hbm.at[r, pl.ds(0, 2 * D)], 17 + t)

    def dsc_pair(j, c_):
        c0 = 2 * j * D
        dm = rowbuf[0:1, pl.ds(_mo(c0, 128), 2 * D)]
        dsc_ref[...] += _dot(jnp.broadcast_to(dm[:, 0:D], (16, D)).astype(bf16),
                             wmod_buf[:, pl.ds(_mo(c0, 128), D)], NT)
        chain = _Chain(j)
        dm8 = rowbuf[:, pl.ds(_mo(c0 + D, 128), D)]
        for r in range(0, D, 32):
            w = wmod_buf[r:r + 32, pl.ds(_mo(c0 + D, 128), D)].astype(f32)
            dmt = jnp.concatenate([chain.tie(dm8[:, n * 128:(n + 1) * 128], 32) for n in range(5)], axis=1)
            a = dscT[r:r + 32, :] + _fold(w * dmt)
            chain.push(_vsum(a))
            dscT[r:r + 32, :] = a
        return c_

    def dmod_pair(j, c_):
        cs = pl.ds(_mo(j * 2 * D, 128), 2 * D)
        dm = rowbuf[0:1, cs]
        for r in range(0, D, 32):
            st_mod[r:r + 32, cs] = (_rep(scT[r:r + 32, :], 2 * D) * dm).astype(bf16)
        o_mod(j).start()
        return c_

    r40 = _iota((40, 128), 0)
    hmask = [jnp.logical_and(r40 >= 10 * j, r40 < 10 * j + 10) for j in range(4)]

    def segment(it, carry):
        s = NSEG - 1 - it
        r0 = _mo(s * (D // 2), 8)
        tok = pl.ds(_mo(s * L, L), L)
        last = it == NSEG - 1
        prev = lambda a: jnp.where(it == 0, 0.0, a)

        hb = _B(h1T[pl.ds(r0, D // 2), :])
        q = _dot(_B(wqoT[0:D // 2, :]), hb, NN)
        qT[...] = _pack(q)
        qsT[...] = _pack(q * (SCALE * LOG2E))
        pqT[0:D // 2, :] = _pack(_phi(q))
        r16 = _iota((16, L), 0)

        def build_kv(i):
            k_u = kT[pl.ds(r0 + i * 40, 40), :]
            v_u = vT[pl.ds(r0 + i * 40, 40), :]
            knat[i * 256:(i + 1) * 256, :] = _U(_B(jnp.concatenate([k_u, zeros24], axis=0)).T)
            vnat[i * 256:(i + 1) * 256, :] = _U(_B(jnp.concatenate([v_u, ones24], axis=0)).T)
            for j in range(4):
                keep = jnp.logical_and(r16 >= 2 * j, r16 < 2 * j + 10)
                vaug[(4 * i + j) * 16:(4 * i + j + 1) * 16, :] = jnp.where(keep, v_u[8 * j:8 * j + 16], ONES_U)

        def score_tile(nat, i, t, u, w):
            b0 = i * 256 + u * 64
            if u != t:
                return _dot(_B(nat[pl.ds(_mo(b0, 8), 64), :]), _B(jnp.concatenate(w, axis=1)), NN)
            lo = _iota((64, 128), 1) < 64
            top = _dot(_B(nat[pl.ds(_mo(b0, 8), 32), :]), _B(jnp.concatenate(w, axis=1)), NN)
            w2 = jnp.concatenate([jnp.where(lo, w[0], w[1]), jnp.where(lo, w[2], w[3])], axis=1)
            bot = _dot(_B(nat[pl.ds(_mo(b0 + 32, 8), 32), :]), _B(w2), NN)
            bot = jnp.concatenate([bot[:, 0:128], bot[:, 0:128], bot[:, 128:256], bot[:, 128:256]], axis=1)
            return jnp.concatenate([top, bot], axis=0)

        def s_tile(i, t, u, mx):
            qt = qsT[pl.ds(_mo(i * 40, 8), 40), t * 128:(t + 1) * 128]
            qt = (_swap(qt), qt)
            w = [jnp.concatenate([jnp.where(hmask[j], qt[j % 2], jnp.uint32(0)), zeros24[:, 0:128]], axis=0)
                 for j in range(4)]
            sc_ = score_tile(knat, i, t, u, w)
            if u == t:
                lane = _iota((128, 128), 1)
                causal = (_iota((128, 128), 0) <= (lane ^ 64), _iota((128, 128), 0) <= lane)
                sc_ = jnp.concatenate([jnp.where(causal[j % 2], sc_[:, j * 128:(j + 1) * 128], -1e30)
                                       for j in range(4)], axis=1)
            sbuf[2 * POFF[t] + u * 128:2 * POFF[t] + (u + 1) * 128, :] = sc_
            for k in range(16):
                v = sc_[8 * k:8 * k + 8]
                mx = v if mx is None else jnp.maximum(mx, v)
            if u == t:
                mx = jnp.max(mx, axis=0, keepdims=True)
            return mx

        def p_tile(i, t, u, mx, ws):
            for j in range(4):
                lj = slice(j * 128, (j + 1) * 128)
                sj = sbuf[2 * POFF[t] + u * 128:2 * POFF[t] + (u + 1) * 128, lj]
                p = jnp.exp2(sj - mx[:, lj]).astype(bf16)
                p_ref[pl.ds(_mo(i * 640 + POFF[t] + u * 64, 8), 64), lj] = _U(p)
                va = _B(vaug[pl.ds(_mo((i * 4 + j) * 16, 16), 16), u * 128:(u + 1) * 128])
                w = _dot(va, p, NN)
                ws[j] = w if ws[j] is None else ws[j] + w
            if u == t:
                ws = [_swap(ws[0]), ws[1], _swap(ws[2]), ws[3]]
                ls = [1.0 / (ws[j][24:32] if j < 2 else ws[j][0:8]) for j in range(4)]
                linv = _assemble_rows(ls)
                rq = pl.ds(_mo(i * QR, 8), QR)
                lt = slice(t * 128, (t + 1) * 128)
                ad = _assemble(ws) * linv
                adot[rq, lt] = ad
                g = gT_ref[rq, :]
                cinv[rq, lt] = linv * (1.0 - g)
                o = g * amem[rq, lt] + (1.0 - g) * ad
                oT[pl.ds(_mo(i * 40, 8), 40), lt] = _pack(o)

        mx_first = None
        for i in range(NQ):
            build_kv(i)
            if i == QP:
                for u in range(4):
                    mx_first = s_tile(0, 3, u, mx_first)

        def attn_fwd(i, mx3):
            i_next = jnp.minimum(i + 1, NQ - 1)
            mx = {3: mx3, 2: None, 1: None, 0: None, 4: None}
            ws = {t: [None] * 4 for t in range(4)}
            s_jobs = [(2, 0), (2, 1), (2, 2), (1, 0), (1, 1), (0, 0), (4, 0), (4, 1), (4, 2), (4, 3)]
            p_jobs = [(3, 0), (3, 1), (3, 2), (3, 3), (2, 0), (2, 1), (2, 2), (1, 0), (1, 1), (0, 0)]
            def mem_read():
                rq = pl.ds(_mo(i * QR, 8), QR)
                mm = m_state[pl.ds(_mo(s * D + i * QR, 8), QR), :]
                mt = jnp.concatenate([mm, jnp.zeros((48, 128), f32)], axis=0).T
                zh = jnp.where((_iota((32, 128), 0) // 8) == (_iota((32, 128), 1) // DH), mt[QR:QR + 32], 0.0)
                lhs = jnp.concatenate([jnp.where(bd, mt[0:QR], 0.0), zh], axis=0).astype(bf16)
                pq_w = _B(jnp.concatenate([pqT[pl.ds(_mo(i * 40, 8), 40), :], zeros24], axis=0))
                nd = _dot(lhs, pq_w, NN)
                rd = 1.0 / (nd[QR:] + 1e-6)
                rd = _assemble_rows([rd[8 * j:8 * j + 8] for j in range(4)])
                amem[rq, :] = nd[0:QR] * rd
                rden[rq, :] = _rep(gT_ref[rq, :]) * rd

            for n_, ((st, su), (pt, pu)) in enumerate(zip(s_jobs, p_jobs)):
                if n_ == MPOS:
                    mem_read()
                if st == 4:
                    mx[4] = s_tile(i_next, 3, su, mx[4])
                else:
                    mx[st] = s_tile(i, st, su, mx[st])
                p_tile(i, pt, pu, mx[pt], ws[pt])
            return mx[4]

        with _scope("attn_fwd"):
            _loop(NQ, attn_fwd, mx_first, UF)

        dyT[...] = _U(dy_buf[tok, :].T)
        chain = _Chain(it)
        for r in range(0, D, RC):
            gb = modT[5 * D + r:5 * D + r + RC, :]
            gb = jnp.concatenate([chain.tie(gb[0:8], 8), gb[8:]], axis=0)
            dffn = _B(dyT[r // 2:(r + RC) // 2, :]).astype(f32) * _rep(gb)
            dffnT[r // 2:(r + RC) // 2, :] = _pack(dffn)
            db = acc_vec[6 * D + r:6 * D + r + RC, :] + _fold(dffn)
            chain.push(db[0:8])
            acc_vec[6 * D + r:6 * D + r + RC, :] = db
        chain0 = chain
        attn = _dot(_B(wqoT[D // 2:D, :]), _B(oT[...]), NN)
        for t in range(4):
            lt = slice(t * 128, (t + 1) * 128)
            acc = chain0.tie(jnp.zeros((8, 128), f32), 8) if t == TIE0 else None
            for r in range(0, D, RC):
                at = attn[r:r + RC, lt]
                sA[r:r + RC, lt] = at
                x2 = _B(xT[pl.ds(r0 + r // 2, RC // 2), lt]).astype(f32) + modT[2 * D + r:2 * D + r + RC, :] * at
                sB[r:r + RC, lt] = x2
                acc = _vsum(x2, acc)
            mu2 = jnp.sum(acc, axis=0, keepdims=True) * (1.0 / D)
            accs = [None] * (1 if t < 3 else 4)
            for n, r in enumerate(range(0, D, RC)):
                xc2 = sB[r:r + RC, lt] - mu2
                accs[n % len(accs)] = _vsum(xc2 * xc2, accs[n % len(accs)])
            acc = _vsum(jnp.concatenate(accs, axis=0))
            rstd2 = jax.lax.rsqrt(jnp.sum(acc, axis=0, keepdims=True) * (1.0 / D) + EPS)
            stat2[:, lt] = jnp.broadcast_to(rstd2, (8, 128))
            mu2 = jnp.broadcast_to(mu2, (8, 128))
            chain = _Chain(it, 1 if t < 3 else LAGT)
            for r in range(0, D, RC):
                xh2 = (sB[r:r + RC, lt] - chain.tie(mu2, RC)) * rstd2
                sC[r:r + RC, lt] = xh2
                h2 = xh2 * modT[4 * D + r:4 * D + r + RC, :] + modT[3 * D + r:3 * D + r + RC, :]
                chain.push(h2)
                h2T[r // 2:(r + RC) // 2, lt] = _pack(h2)

        def ffn_chunk(ci, c_):
            rp = pl.ds(_mo(ci * (FCH // 2), 8), FCH // 2)
            rf = pl.ds(_mo(ci * FCH, 16), FCH)
            h2b = _B(h2T[...])
            dfb = _B(dffnT[...])
            u = _dot(w1_buf[rf, :], h2b, NN) + _rep(b1T[rf, :])
            dg = _dot(w2_buf[rf, :], dfb, NN)
            u2 = u * u
            th = jnp.tanh(u * (GELU_C1 + GELU_C2 * u2))
            hp = 0.5 * th + 0.5
            gactT[rp, :] = _pack(u * hp)
            gp = hp + (0.5 * u) * (1.0 - th * th) * (GELU_C1 + (3.0 * GELU_C2) * u2)
            du = dg * gp
            duT[rp, :] = _pack(du)
            acc_vec[pl.ds(_mo(7 * D + ci * FCH, 8), FCH), :] += _fold(du)
            a2 = prev(acc_w2[rf, :]) + _dot(_B(gactT[rp, :]), dfb, NT)
            acc_w2[rf, :] = a2
            st_w2[rf, :] = a2.astype(bf16)
            a1 = prev(acc_w1T[rf, :]) + _dot(_B(duT[rp, :]), h2b, NT)
            acc_w1T[rf, :] = a1
            st_w1[rf, :] = a1.astype(bf16)
            for blk in (ci, ci + NFC, jnp.minimum(ci + 2 * NFC, FP // 128 - 1)):
                rb = pl.ds(_mo(blk * 128, 128), 128)
                w1N[:, rb] = _U(w1_buf[rb, :].T)
                w2T[:, rb] = _U(w2_buf[rb, :].T)
            return c_

        with _scope("ffn_chunk"):
            _loop(NFC, ffn_chunk, 0, UC)

        @pl.when(last)
        def _():
            o_w1.start()
            o_w2.start()

        def post_ffn(hf, c_):
            hl = pl.ds(_mo(hf * HL, HL), HL)
            rows = pl.ds(_mo(s * L + hf * HL, HL), HL)
            dh2 = _dot(_B(w1N[...]), _B(duT[:, hl]), NN)
            for t in range(2):
                lt = pl.ds(_mo(hf * HL + t * 128, 128), 128)
                s1 = s2 = None
                for r in range(0, D, RC):
                    dh = dh2[r:r + RC, t * 128:(t + 1) * 128]
                    xh2 = sC[r:r + RC, lt]
                    acc_vec[3 * D + r:3 * D + r + RC, :] += dh
                    acc_vec[4 * D + r:4 * D + r + RC, :] += dh * xh2
                    dxh = dh * modT[4 * D + r:4 * D + r + RC, :]
                    sD[r:r + RC, lt] = dxh
                    s1 = _vsum(dxh, s1)
                    s2 = _vsum(dxh * xh2, s2)
                m1 = jnp.sum(s1, axis=0, keepdims=True) * (1.0 / D)
                m2 = jnp.sum(s2, axis=0, keepdims=True) * (1.0 / D)
                rs = stat2[0:1, lt]
                m1 = jnp.broadcast_to(m1, (8, 128))
                chain = _Chain(hf)
                for r in range(0, D, RC):
                    dx2 = _B(dyT[r // 2:(r + RC) // 2, lt]).astype(f32) + rs * (
                        sD[r:r + RC, lt] - chain.tie(m1, RC) - sC[r:r + RC, lt] * m2)
                    chain.push(dx2)
                    sD[r:r + RC, lt] = dx2
                    acc_vec[2 * D + r:2 * D + r + RC, :] += dx2 * sA[r:r + RC, lt]
                    dffnT[r // 2:(r + RC) // 2, lt] = _pack(dx2 * modT[2 * D + r:2 * D + r + RC, :])

            def ffn_part(lo, hi):
                ffn = _dot(_B(w2T[lo // 2:hi // 2, :]), _B(gactT[:, hl]), NN) + _rep(b2T[lo:hi, :], HL)
                acc_vec[5 * D + lo:5 * D + hi, :] += _fold(_B(dyT[lo // 2:hi // 2, hl]).astype(f32) * ffn)
                outT = sB[lo:hi, hl] + _rep(modT[5 * D + lo:5 * D + hi, :], HL) * ffn
                x_buf[rows, lo:hi] = outT.astype(bf16).T

            ffn_part(0, _FSPLIT)
            do_all = _dot(wqkv_buf[3], _B(dffnT[:, hl]), NN)
            if _FSPLIT < D:
                ffn_part(_FSPLIT, D)
            for i in range(NQ):
                rq = slice(i * QR, (i + 1) * QR)
                do = do_all[rq]
                ad = adot[rq, hl]
                am = amem[rq, hl]
                acc_vec[10 * D + i * QR:10 * D + (i + 1) * QR, :] += _fold(do * (am - ad))
                dOp[i * 72:i * 72 + 40, hl] = _pack(do * cinv[rq, hl])
                parts = _head_partials(_B(dOp[i * 72:i * 72 + 40, hl]).astype(f32) * ad)
                for j in range(4):
                    hi = (-parts[j]).astype(bf16).astype(f32)
                    lo = -parts[j] - hi
                    dOp[i * 72 + 40 + 8 * j:i * 72 + 48 + 8 * j, hl] = _pack(jnp.concatenate([hi, lo], axis=0))
                dnum = do * rden[rq, hl]
                tp = _head_partials(dnum * am)
                wmemT[i * 56:(i + 1) * 56, hl] = _pack(jnp.concatenate([dnum] + [-x for x in tp], axis=0))
            out_copy(s, hf).start()
            return c_

        with _scope("post_ffn"):
            jax.lax.fori_loop(0, 2, post_ffn, 0)

        def attn_bwd(i, c_):
            rq = pl.ds(_mo(i * QR, 8), QR)
            rp = pl.ds(_mo(i * 40, 8), 40)
            d0 = _mo(i * 72, 8)
            dq = [[None] * 4 for _ in range(4)]
            dk = [[None] * 4 for _ in range(4)]
            dv = [[None] * 4 for _ in range(4)]
            mem = {}
            lhs = {}

            def wmem():
                return _B(jnp.concatenate([wmemT[pl.ds(_mo(i * 56, 8), 56), :], jnp.zeros((8, L), u32)], axis=0))

            def mem_dq():
                mm = m_state[pl.ds(_mo(s * D + i * QR, 8), QR), :]
                dpq = _dot(jnp.where(mask2, mm, 0.0).astype(bf16), wmem(), NN)
                qq = _B(qT[rp, :]).astype(f32)
                mem['q'] = dpq * jnp.where(qq > 0, 1.0, _B(pqT[rp, :]).astype(f32))

            def mem_dkv():
                kk = _B(kT[pl.ds(r0 + i * 40, 40), :]).astype(f32)
                pk = _phi(kk)
                pk_w = jnp.concatenate([pk, jnp.zeros((48, L), f32)], axis=0).astype(bf16)
                v_aug = _B(jnp.concatenate([vT[pl.ds(r0 + i * 40, 40), :], ones24], axis=0))
                dms = dm_state[rq, :]
                dpk = _dot(jnp.where(mask2, dms, 0.0).astype(bf16), v_aug, NN)
                dmt = jnp.concatenate([jnp.where(bd, dms, 0.0), jnp.zeros((48, 128), f32)], axis=0).T
                mem['v'] = _dot(dmt[0:QR].astype(bf16), pk_w, NN)
                mem['k'] = dpk * jnp.where(kk > 0, 1.0, pk)

            def mem_update():
                dm_state[rq, :] += _dot(_B(pqT[rp, :]), wmem(), NT)

            def dp_tile(t, u):
                lt = slice(t * 128, (t + 1) * 128)
                dt = dOp[pl.ds(d0, 72), lt]
                dt = (_swap(dt), dt)
                wd = [jnp.concatenate([jnp.where(hmask[j], dt[j % 2][0:40], jnp.uint32(0)),
                                       dt[j % 2][40 + 8 * j:48 + 8 * j], jnp.zeros((16, 128), u32)], axis=0)
                      for j in range(4)]
                dp = score_tile(vnat, i, t, u, wd)
                res = []
                for j in range(4):
                    p = _B(p_ref[pl.ds(_mo(i * 640 + POFF[t] + u * 64, 8), 64), j * 128:(j + 1) * 128])
                    res.append((dp[:, j * 128:(j + 1) * 128] * p.astype(f32)).astype(bf16))
                return res

            def thin_tile(t, u, ds):
                lt = slice(t * 128, (t + 1) * 128)
                for j in range(4):
                    p = _B(p_ref[pl.ds(_mo(i * 640 + POFF[t] + u * 64, 8), 64), j * 128:(j + 1) * 128])
                    kw = _B(kT[pl.ds(r0 + i * 40 + 8 * j, 16), u * 128:(u + 1) * 128])
                    if (t, j) not in lhs:
                        qw = qT[pl.ds(_mo(i * 40 + 8 * j, 8), 16), lt]
                        dw = dOp[pl.ds(d0 + 8 * j, 16), lt]
                        if j % 2 == 0:
                            qw, dw = _swap(qw), _swap(dw)
                            lhs[(t, j)] = (qw, dw)
                    else:
                        qw, dw = lhs[(t, j)]
                    qw, dw = _B(qw), _B(dw)
                    b = _dot(dw, p, NT)
                    a = _dot(qw, ds[j], NT)
                    e = _dot(kw, ds[j], NN)
                    dq[j][t] = e if dq[j][t] is None else dq[j][t] + e
                    dk[j][u] = a if dk[j][u] is None else dk[j][u] + a
                    dv[j][u] = b if dv[j][u] is None else dv[j][u] + b
                if u == t:
                    col = lambda w: _assemble([w[j][t] for j in range(4)])
                    dq[0][t], dq[2][t] = _swap(dq[0][t]), _swap(dq[2][t])
                    dqkvT[rp, lt] = _pack(col(dq) * SCALE + mem['q'][:, lt])
                    dqkvT[pl.ds(_mo(D // 2 + i * 40, 8), 40), lt] = _pack(col(dk) * SCALE + mem['k'][:, lt])
                    dqkvT[pl.ds(_mo(D + i * 40, 8), 40), lt] = _pack(col(dv) + mem['v'][:, lt])

            jobs = [(t, u) for t in (3, 2, 1, 0) for u in range(t + 1)]
            def dwo(n):
                def f():
                    cs = slice(n * 128, (n + 1) * 128)
                    r16 = pl.ds(_mo(i * QR, 16), QR)
                    ao = prev(acc_wo[rq, cs]) + _dot(_B(oT[rp, :]), _B(dffnT[n * 64:(n + 1) * 64, :]), NT)
                    acc_wo[rq, cs] = ao
                    st_w[3, r16, cs] = ao.astype(bf16)
                return f

            def rowsums():
                rowbuf[:, pl.ds(_mo(2 * D + i * D, 128), D)] = jnp.broadcast_to(
                    _rowsum(acc_vec[pl.ds(_mo(2 * D + i * D, 8), D), :]), (8, D))

            extra = {0: [mem_dq], 1: [mem_dkv], 9: [mem_update]}
            extra.setdefault(RSP, []).append(rowsums)
            for n, pos in enumerate(_DWO_POS):
                extra.setdefault(pos, []).append(dwo(n))
            for f in extra.get(-1, []):
                f()
            ds = dp_tile(*jobs[0])
            for n_, job in enumerate(jobs):
                ds_next = dp_tile(*jobs[n_ + 1]) if n_ + 1 < len(jobs) else None
                for f in extra.get(n_, []):
                    f()
                thin_tile(job[0], job[1], ds)
                ds = ds_next
            for f in extra.get(10, []):
                f()
            return c_

        with _scope("attn_bwd"):
            _loop(NQ, attn_bwd, 0, UB)

        @pl.when(last)
        def _():
            o_wo.start()
            b2_buf[...] = rowbuf[0:1, 6 * D:7 * D].reshape(D).astype(bf16)
            o_b2.start()
            b1_buf[...] = rowbuf[0:1, 7 * D:7 * D + F].reshape(F).astype(bf16)
            o_b1.start()
            jax.lax.fori_loop(1, 3, dmod_pair, 0)

        def dw_chunk(t):
            ra = pl.ds(_mo(t * WCH, 16), WCH)
            aw = prev(acc_wqkv[ra, :]) + _dot(_B(h1T[pl.ds(r0 + t * (WCH // 2), WCH // 2), :]), _B(dqkvT[...]), NT)
            acc_wqkv[ra, :] = aw
            for k in range(3):
                st_w[k, ra, :] = aw[:, k * D:(k + 1) * D].astype(bf16)

            @pl.when(last)
            def _():
                for k in range(3):
                    o_w(k, t).start()

        def qkv_bwd_a(a, c_):
            hl = pl.ds(_mo(a * HL, HL), HL)
            dh1 = _dot(wqkv_buf[0], _B(dqkvT[0:D // 2, hl]), NN)
            dh1 = dh1 + _dot(wqkv_buf[1], _B(dqkvT[D // 2:D, hl]), NN)
            dh1 = dh1 + _dot(wqkv_buf[2], _B(dqkvT[D:3 * D // 2, hl]), NN)
            for t in range(2):
                lt = pl.ds(_mo(a * HL + t * 128, 128), 128)
                mu = stat1[pl.ds(_mo(s * 16, 8), 1), lt]
                rstd = stat1[pl.ds(_mo(s * 16 + 8, 8), 1), lt]
                xh = lambda r: (_B(xT[pl.ds(r0 + r // 2, RC // 2), lt]).astype(f32) - mu) * rstd
                s1 = s2 = None
                for r in range(0, D, RC):
                    dh = dh1[r:r + RC, t * 128:(t + 1) * 128]
                    xh1 = xh(r)
                    acc_vec[r:r + RC, :] += dh
                    acc_vec[D + r:D + r + RC, :] += dh * xh1
                    dxh = dh * modT[D + r:D + r + RC, :]
                    sA[r:r + RC, lt] = dxh
                    s1 = _vsum(dxh, s1)
                    s2 = _vsum(dxh * xh1, s2)
                m1 = jnp.broadcast_to(jnp.sum(s1, axis=0, keepdims=True) * (1.0 / D), (8, 128))
                m2 = jnp.sum(s2, axis=0, keepdims=True) * (1.0 / D)
                chain = _Chain(a)
                for r in range(0, D, RC):
                    dx = _pack(sD[r:r + RC, lt] + rstd * (sA[r:r + RC, lt] - chain.tie(m1, RC) - xh(r) * m2))
                    chain.push(pltpu.bitcast(dx, f32))
                    dyT[r // 2:(r + RC) // 2, lt] = dx
                dy_buf[pl.ds(_mo(s * L + a * HL + t * 128, 128), 128), :] = _B(dyT[:, lt]).T
            dw_chunk(a)
            dx_copy(s, a).start()
            return c_

        def qkv_bwd_b(b, c_):
            dw_chunk(2 + b)
            return c_

        with _scope("qkv_bwd_a"):
            jax.lax.fori_loop(0, 2, qkv_bwd_a, 0)

        @pl.when(last)
        def _():
            dm = _rowsum(acc_vec[0:2 * D, :])

            def piece(t, c_):
                r = pl.ds(_mo(t * WCH, 16), WCH)
                st_mod[r, 0:2 * D] = (_rep(scT[r, :], 2 * D) * dm).astype(bf16)
                o_mod01(t).start()
                return c_

            jax.lax.fori_loop(0, 4, piece, 0)
            rowbuf[:, 0:2 * D] = jnp.broadcast_to(dm, (8, 2 * D))

        with _scope("qkv_bwd_b"):
            jax.lax.fori_loop(0, 2, qkv_bwd_b, 0)

        return carry

    with _scope("segment"):
        jax.lax.fori_loop(0, NSEG, segment, 0)

    gate = gate_row()
    dgc = jnp.sum(acc_vec[10 * D:11 * D, :], axis=1, keepdims=True)
    dgate = jnp.sum(jnp.where(head_onehot(), jnp.broadcast_to(dgc, (D, H)), 0.0), axis=0, keepdims=True)
    beta_buf[...] = (dgate * gate * (1.0 - gate)).reshape(H).astype(bf16)
    o_beta.start()
    jax.lax.fori_loop(0, 3, dsc_pair, 0)
    c_, sig = silu_parts()
    dsc = dsc_ref[0:1, :] + _rowsum(dscT[...])
    c_buf[...] = (dsc * (sig * (1.0 + c_ * (1.0 - sig)))).astype(bf16)
    o_c.start()

    with _scope("wait1"):
        for s in range(NSEG):
            for hf in range(2):
                out_copy(s, hf).wait()
                dx_copy(s, hf).wait()
        for d in [o_w2, o_w1, o_wo, o_b1, o_b2] + [o_mod(k) for k in range(1, 3)] + [
                o_w(k, t) for k in range(3) for t in range(4)]:
            d.wait()
    with _scope("wait2"):
        o_mod01(0).wait()
        o_mod01(1).wait()
    with _scope("wait3"):
        o_mod01(2).wait()
        o_mod01(3).wait()
    with _scope("wait4"):
        o_c.wait()
        o_beta.wait()


@jax.jit
def pallas_adaLN_cond__memory_aug_infini_attn__dense_activation_gelu__prompt_kernel(
    A_x: jax.Array,
    A_wq: jax.Array,
    A_wk: jax.Array,
    A_wv: jax.Array,
    A_wo: jax.Array,
    A_beta: jax.Array,
    B_x: jax.Array,
    B_w1: jax.Array,
    B_b1: jax.Array,
    B_w2: jax.Array,
    B_b2: jax.Array,
    c: jax.Array,
    w_mod: jax.Array,
    grad_out: jax.Array,
):
    del B_x
    hbm = pl.BlockSpec(memory_space=pltpu.HBM)
    sds = jax.ShapeDtypeStruct
    V = pltpu.VMEM
    scratch = [
        V((S, D), bf16), V((S, D), bf16), V((4, D, D), bf16), V((FP, D), bf16),
        V((FP, D), bf16), V((D, 6 * D), bf16),
        V((H,), bf16), V((F,), bf16), V((D,), bf16), V((1, D), bf16),
        V((F, D), bf16), V((F, D), bf16), V((4, D, D), bf16),
        V((D, D), u32), V((D, D), u32), V((D // 2, FP), u32), V((D // 2, FP), u32),
        V((8 * D, 128), f32), V((F, 128), f32), V((D, 128), f32), V((D, 128), f32), V((D, 128), f32),
        V((16, D), f32), V((D, 128), f32), V((D, 6 * D), bf16),
        V((NSEG * D // 2, L), u32), V((D // 2, L), u32), V((NSEG * 16, L), f32),
        V((NSEG * D // 2, L), u32), V((NSEG * D // 2, L), u32),
        V((NSEG * D // 2, L), u32), V((8, L), f32),
        V(((NSEG + 1) * D, 128), f32), V((D, 128), f32),
        V((D // 2, L), u32), V((D // 2, L), u32), V((D // 2, L), u32),
        V((NQ * 256, 128), u32), V((NQ * 256, 128), u32), V((H * 16, L), u32), V((NQ * 640, L), u32), V((1280, L), f32),
        V((D, L), f32), V((D, L), f32), V((D, L), f32), V((D, L), f32), V((D // 2, L), u32),
        V((D, L), f32), V((D, L), f32), V((D, L), f32), V((D, L), f32),
        V((D // 2, L), u32), V((D // 2, L), u32), V((D // 2, L), u32), V((FP // 2, L), u32), V((FP // 2, L), u32),
        V((NQ * 72, L), u32), V((NQ * 56, L), u32), V((3 * D // 2, L), u32),
        V((D, 3 * D), f32), V((D, D), f32), V((F, D), f32), V((F, D), f32), V((11 * D, 128), f32),
        V((8, 10 * D), f32),
        pltpu.SemaphoreType.DMA((61,)),
    ]
    outs = pl.pallas_call(
        _kernel,
        in_specs=[hbm] * 13,
        out_specs=[hbm] * 13,
        out_shape=[
            sds((1, S, D), bf16), sds((1, S, D), bf16), sds((D, D), bf16), sds((D, D), bf16),
            sds((D, D), bf16), sds((D, D), bf16), sds((H,), bf16), sds((F, D), bf16), sds((F,), bf16),
            sds((F, D), bf16), sds((D,), bf16), sds((1, D), bf16), sds((D, 6 * D), bf16),
        ],
        scratch_shapes=scratch,
        compiler_params=pltpu.CompilerParams(vmem_limit_bytes=124 * 1024 * 1024),
    )(A_x, A_wq, A_wk, A_wv, A_wo, A_beta, B_w1.T, B_b1, B_w2, B_b2, c, w_mod, grad_out)
    out, dx, dwq, dwk, dwv, dwo, dbeta, dw1, db1, dw2, db2, dc, dwmod = outs
    return (out, dx, dwq, dwk, dwv, dwo, dbeta, dw1.T, db1, dw2, db2, dc, dwmod)
```

```python
import contextlib
import math

import jax
import jax.numpy as jnp
import jax.experimental.pallas as pl
import jax.experimental.pallas.tpu as pltpu

bf16 = jnp.bfloat16
f32 = jnp.float32
u32 = jnp.uint32

S, D, H, DH, NSEG, L, F = 2048, 640, 32, 20, 4, 512, 1728
FP = 1792
NQ = 8
QR = 80
FCH = 288
NFC = F // FCH
SCALE = DH ** -0.5
LOG2E = math.log2(math.e)
GELU_C1 = math.sqrt(2.0 / math.pi)
GELU_C2 = GELU_C1 * 0.044715
EPS = 1e-5
POFF = (0, 64, 192, 384)

_PROFILE = False
QP = 7
QP2 = 0
QS = 320
RSP = 3
ML = 1
UF, UB, UC = 2, 4, 2
MPOS = 3
TIE0 = 0
LAGT = 4
RC = 16
RC0 = 32
_FSPLIT = 640
_DWO_POS = (2, 4, 6, 7, 8)


def _scope(name):
    return jax.named_scope(name) if _PROFILE else contextlib.nullcontext()


NN = (((1,), (0,)), ((), ()))
NT = (((1,), (1,)), ((), ()))


def _dot(a, b, dims):
    return jax.lax.dot_general(a, b, dims, preferred_element_type=f32)


def _B(x):
    return pltpu.bitcast(x, bf16)


def _U(x):
    return pltpu.bitcast(x, u32)


def _pack(x):
    return _U(x.astype(bf16))


def _iota(shape, dim):
    return jax.lax.broadcasted_iota(jnp.int32, shape, dim)


def _rep(p, n=L):
    return jnp.concatenate([p] * (n // 128), axis=1)


def _fold(x):
    acc = x[:, 0:128]
    for t in range(1, x.shape[1] // 128):
        acc = acc + x[:, t * 128:(t + 1) * 128]
    return acc


def _vsum(x, acc=None):
    for k in range(x.shape[0] // 8):
        v = x[8 * k:8 * k + 8]
        acc = v if acc is None else acc + v
    return acc


class _Chain:
    def __init__(self, idx, lag=1):
        self.lag = lag
        self.true = None if idx is None else _iota((8, 128), 0) >= jnp.minimum(idx, 0)
        self.done = []

    def tie(self, x, rows):
        if self.true is not None and len(self.done) >= self.lag:
            x = jnp.where(self.true, x, self.done[-self.lag])
        return jnp.concatenate([x] * (rows // 8), axis=0)

    def push(self, y):
        self.done.append(y[y.shape[0] - 8:, 0:128])


def _loop(n, body, init, unroll):
    def wide(i, c):
        for k in range(unroll):
            c = body(i * unroll + k, c)
        return c
    return jax.lax.fori_loop(0, n // unroll, wide, init)


def _colrep(row):
    return jnp.broadcast_to(row, (128, row.shape[1])).T


def _rowsum(acc):
    return jnp.sum(acc.T, axis=0, keepdims=True)


def _phi(x):
    return jnp.where(x > 0, x + 1.0, jnp.exp(x))


def _mo(x, m):
    return pl.multiple_of(x, m)


def _rot(x, j):
    return x if j % 2 else pltpu.roll(x, 64, 1)


def _lt(t):
    return slice(t * 128, (t + 1) * 128) if isinstance(t, int) else pl.ds(_mo(t * 128, 128), 128)


def _assemble(w):
    lo = _iota((8, w[0].shape[1]), 0) < 4
    return jnp.concatenate([
        w[0][0:16], jnp.where(lo, w[0][16:24], w[1][0:8]), w[1][8:24],
        w[2][8:24], jnp.where(lo, w[2][24:32], w[3][8:16]), w[3][16:32]], axis=0)


def _assemble_rows(r):
    lo = _iota(r[0].shape, 0) < 4
    return jnp.concatenate([
        r[0], r[0], jnp.where(lo, r[0], r[1]), r[1], r[1],
        r[2], r[2], jnp.where(lo, r[2], r[3]), r[3], r[3]], axis=0)


def _head_partials(x):
    lo = _iota((8, x.shape[1]), 0) < 4
    v = [x[8 * k:8 * k + 8] for k in range(10)]
    return [v[0] + v[1] + jnp.where(lo, v[2], 0.0),
            jnp.where(lo, 0.0, v[2]) + v[3] + v[4],
            v[5] + v[6] + jnp.where(lo, v[7], 0.0),
            jnp.where(lo, 0.0, v[7]) + v[8] + v[9]]


def _kernel(x_hbm, wq_hbm, wk_hbm, wv_hbm, wo_hbm, beta_hbm, w1_hbm, b1_hbm, w2_hbm, b2_hbm,
            c_hbm, wmod_hbm, dy_hbm,
            out_hbm, dx_hbm, dwq_hbm, dwk_hbm, dwv_hbm, dwo_hbm, dbeta_hbm, dw1_hbm, db1_hbm,
            dw2_hbm, db2_hbm, dc_hbm, dwmod_hbm,
            x_buf, dy_buf, wqkv_buf, w1_buf, w2_buf, wmod_buf,
            beta_buf, b1_buf, b2_buf, c_buf,
            st_w1, st_w2, st_w,
            wqoT, wkvT, w1N, w2T,
            modT, b1T, b2T, gT_ref, scT, dsc_ref, dscT, st_mod,
            xT, hnext, stat1, h1T, kT, vT, stat2,
            m_state, dm_state,
            qT, qsT, pqT, knat, vnat, vaug, p_ref, sbuf,
            adot, amem, rden, cinv, oT, sA, sB, sC, sD,
            h2T, dffnT, dyT, gactT, duT, dOp, wmemT, dqkvT,
            acc_wqkv, acc_wo, acc_w1T, acc_w2, acc_vec, rowbuf,
            sems):
    def cp(src, dst, k):
        return pltpu.make_async_copy(src, dst, sems.at[k])

    def in_x(s):
        r = pl.ds(_mo(s * L, L), L)
        return cp(x_hbm.at[0, r, :], x_buf.at[r, :], 1 + s)

    in_wmodA = cp(wmod_hbm.at[:, pl.ds(0, 2 * D)], wmod_buf.at[:, pl.ds(0, 2 * D)], 0)
    in_w = {0: cp(wq_hbm, wqkv_buf.at[0], 5), 2: cp(wv_hbm, wqkv_buf.at[2], 7), 3: cp(wo_hbm, wqkv_buf.at[3], 9)}
    in_wmodB = cp(wmod_hbm.at[:, pl.ds(2 * D, 4 * D)], wmod_buf.at[:, pl.ds(2 * D, 4 * D)], 8)
    in_w1 = cp(w1_hbm, w1_buf.at[pl.ds(0, F), :], 10)
    in_w2 = cp(w2_hbm, w2_buf.at[pl.ds(0, F), :], 11)
    in_dy = cp(dy_hbm.at[0], dy_buf, 12)
    in_small = [cp(c_hbm, c_buf, 21), cp(beta_hbm, beta_buf, 22), cp(b1_hbm, b1_buf, 23), cp(b2_hbm, b2_buf, 24)]

    for d in in_small:
        d.start()
    in_wk = [cp(wk_hbm.at[pl.ds(lo, n), :], wqkv_buf.at[1, pl.ds(lo, n), :], k)
             for lo, n, k in ((0, 512, 6), (512, 128, 16))]
    for d in [in_x(0), in_w[2], in_wmodA, in_wk[0], in_wk[1], in_x(1), in_w[0], in_x(2), in_w[3],
              in_x(3), in_wmodB, in_dy, in_w1, in_w2]:
        d.start()

    dm_state[...] = jnp.zeros(dm_state.shape, f32)
    m_state[0:D, :] = jnp.zeros((D, 128), f32)
    gactT[F // 2:FP // 2, :] = jnp.zeros(((FP - F) // 2, L), u32)
    duT[F // 2:FP // 2, :] = jnp.zeros(((FP - F) // 2, L), u32)
    w1_buf[F:FP, :] = jnp.zeros((FP - F, D), bf16)
    w2_buf[F:FP, :] = jnp.zeros((FP - F, D), bf16)
    dsc_ref[...] = jnp.zeros(dsc_ref.shape, f32)
    dscT[...] = jnp.zeros(dscT.shape, f32)

    def zero_acc(k, c_):
        acc_vec[pl.ds(_mo(k * D, 8), D), :] = jnp.zeros((D, 128), f32)
        return c_

    jax.lax.fori_loop(0, 11, zero_acc, 0)

    for d in in_small:
        d.wait()

    def silu_parts():
        c = c_buf[...].astype(f32)
        sig_c = 1.0 / (1.0 + jnp.exp(-c))
        return c, sig_c

    def gate_row():
        beta = beta_buf[...].astype(f32).reshape(1, H)
        return 1.0 / (1.0 + jnp.exp(-beta))

    def head_onehot():
        return (_iota((D, H), 0) // DH) == _iota((D, H), 1)

    c, sig_c = silu_parts()
    sc = c * sig_c
    sc16 = jnp.broadcast_to(sc, (16, D)).astype(bf16)
    scT[...] = _colrep(sc.astype(bf16).astype(f32))

    def mod_chunks(lo, hi):
        for k in range(lo, hi):
            m = _dot(sc16, wmod_buf[:, k * D:(k + 1) * D], NN)[0:1, :]
            if k in (1, 4):
                m = m + 1.0
            modT[k * D:(k + 1) * D, :] = _colrep(m)

    def P(k, n=L):
        return _rep(modT[k * D:(k + 1) * D, :], n)

    bd80 = (_iota((QR, 128), 0) // DH) == (_iota((QR, 128), 1) // DH)
    lane80 = _iota((QR, 128), 1)
    bd = jnp.logical_and(bd80, lane80 < QR)
    mask2 = jnp.logical_or(bd, jnp.logical_and(
        jnp.logical_and(lane80 >= QR, lane80 < QR + 32),
        ((lane80 - QR) // 8) == (_iota((QR, 128), 0) // DH)))
    ONES_U = jnp.uint32(0x3F803F80)
    zeros24 = jnp.zeros((24, L), u32)
    ones24 = jnp.full((24, L), ONES_U, u32)

    b1row = b1_buf[...].astype(f32).reshape(1, F)
    for k in range(F // 128):
        b1T[k * 128:(k + 1) * 128, :] = _colrep(b1row[:, k * 128:(k + 1) * 128])
    b1T[F - 128:F, :] = _colrep(b1row[:, F - 128:F])
    b2T[...] = _colrep(b2_buf[...].astype(f32).reshape(1, D))
    gcol = jnp.sum(jnp.where(head_onehot(), jnp.broadcast_to(gate_row(), (D, H)), 0.0), axis=1, keepdims=True)
    gT_ref[...] = jnp.broadcast_to(gcol, (D, 128))

    def x_tile(s, t):
        xt_b = x_buf[pl.ds(_mo(s * L + t * 128, 128), 128), :].T
        xT[pl.ds(_mo(s * (D // 2), 8), D // 2), _lt(t)] = _U(xt_b)

    def ln1_stats(s, t, chain):
        lt = _lt(t)
        ld = lambda r: _B(xT[pl.ds(_mo(s * (D // 2) + r // 2, 8), RC0 // 2), lt]).astype(f32)
        acc = chain.tie(jnp.zeros((8, 128), f32), 8)
        for r in range(0, D, RC0):
            acc = _vsum(ld(r), acc)
        mu = jnp.sum(acc, axis=0, keepdims=True) * (1.0 / D)
        stat1[pl.ds(_mo(s * 16, 8), 8), lt] = jnp.broadcast_to(mu, (8, 128))
        acc = None
        for r in range(0, D, RC0):
            xc = ld(r) - mu
            acc = _vsum(xc * xc, acc)
        rstd = jax.lax.rsqrt(jnp.sum(acc, axis=0, keepdims=True) * (1.0 / D) + EPS)
        stat1[pl.ds(_mo(s * 16 + 8, 8), 8), lt] = jnp.broadcast_to(rstd, (8, 128))
        return jnp.broadcast_to(mu, (8, 128)), rstd

    def ln1_apply(s, t, mu, rstd, chain):
        lt = _lt(t)
        for r in range(0, D, RC0):
            x = _B(xT[pl.ds(_mo(s * (D // 2) + r // 2, 8), RC0 // 2), lt]).astype(f32)
            h = (x - chain.tie(mu, RC0)) * rstd * modT[D + r:D + r + RC0, :] + modT[r:r + RC0, :]
            h = _pack(h)
            chain.push(pltpu.bitcast(h, f32))
            hnext[r // 2:(r + RC0) // 2, lt] = h

    in_x(0).wait()

    def ln0_stats(t, c_):
        x_tile(0, t)
        ln1_stats(0, t, _Chain(None))
        return c_

    def ln0_apply(t, c_):
        ln1_apply(0, t, stat1[0:8, _lt(t)], stat1[8:9, _lt(t)], _Chain(None))
        return c_

    def w_tr(k, r):
        def f(t, c_):
            wkvT[r:r + D // 2, _lt(t)] = _U(wqkv_buf[k, _lt(t), :].T)
            return c_
        return f

    jax.lax.fori_loop(0, 4, ln0_stats, 0)
    in_w[2].wait()
    jax.lax.fori_loop(0, 5, w_tr(2, D // 2), 0)
    in_wmodA.wait()
    mod_chunks(0, 2)
    jax.lax.fori_loop(0, 4, ln0_apply, 0)
    in_wk[0].wait()
    jax.lax.fori_loop(0, 4, w_tr(1, 0), 0)
    in_wk[1].wait()
    w_tr(1, 0)(4, 0)

    def phase0(s, carry):
        @pl.when(s < NSEG - 1)
        def _():
            in_x(s + 1).wait()

        @pl.when(s == 2)
        def _():
            in_w[0].wait()
            in_w[3].wait()
            in_wmodB.wait()

        r0 = _mo(s * (D // 2), 8)
        s_next = jnp.minimum(s + 1, NSEG - 1)
        h1T[pl.ds(r0, D // 2), :] = hnext[...]
        chain = _Chain(s)

        for k in range(4):
            x_tile(s_next, k)
        for k in range(4):
            vv = _dot(_B(wkvT[D // 2 + k * 80:D // 2 + (k + 1) * 80, :]), _B(h1T[pl.ds(r0, D // 2), :]), NN)
            vT[pl.ds(r0 + k * 80, 80), :] = _pack(vv)
            mu, rstd = ln1_stats(s_next, k, chain)
            ln1_apply(s_next, k, mu, rstd, chain)
            kk = _dot(_B(wkvT[k * 80:(k + 1) * 80, :]), _B(h1T[pl.ds(r0, D // 2), :]), NN)
            kT[pl.ds(r0 + k * 80, 80), :] = _pack(kk)
            pqT[0:80, :] = _pack(_phi(kk))
            for i in (2 * k, 2 * k + 1):
                pk_u = pqT[(i % 2) * 40:(i % 2 + 1) * 40, :]
                v_aug = jnp.concatenate([vT[pl.ds(r0 + i * 40, 40), :], ones24], axis=0)
                mm = _dot(_B(pk_u), _B(v_aug), NT)
                b0 = _mo(s * D + i * QR, 8)
                m_state[pl.ds(b0 + D, QR), :] = m_state[pl.ds(b0, QR), :] + mm
        late = s >= 2
        chain2 = _Chain(s, ML)
        src = jnp.where(late, 3 * (s - 2), 1)
        wqoT[pl.ds(_mo((s % 2) * (D // 2), 8), D // 2), :] = _U(wqkv_buf[src].T)
        for j in range(2):
            k = jnp.where(late, 2 * s - 2, 0) + j
            acc = [None] * 5
            for r in range(0, D, RC0):
                w = wmod_buf[r:r + RC0, pl.ds(_mo(k * D, 128), D)].astype(f32)
                for n in range(5):
                    sc_r = jnp.concatenate([chain2.tie(scT[q:q + 8, :], 8) for q in range(r, r + RC0, 8)], axis=0)
                    acc[n] = _vsum(w[:, n * 128:(n + 1) * 128] * sc_r, acc[n])
                    chain2.push(acc[n])
            m = jnp.sum(jnp.concatenate(acc, axis=1), axis=0, keepdims=True) + jnp.where(k == 4, 1.0, 0.0)
            modT[pl.ds(_mo(jnp.where(late, k, 6 + j) * D, 8), D), :] = _colrep(m)
        return carry

    with _scope("phase0"):
        jax.lax.fori_loop(0, NSEG, phase0, 0)

    in_dy.wait()
    in_w1.wait()
    in_w2.wait()

    HL = L // 2

    def out_copy(s, hf):
        r = pl.ds(_mo(s * L + hf * HL, HL), HL)
        return cp(x_buf.at[r, :], out_hbm.at[0, r, :], 25 + 2 * s + hf)

    def dx_copy(s, hf):
        r = pl.ds(_mo(s * L + hf * HL, HL), HL)
        return cp(dy_buf.at[r, :], dx_hbm.at[0, r, :], 33 + 2 * s + hf)

    WCH = D // 4

    def o_w(k, t):
        r = pl.ds(_mo(t * WCH, 16), WCH)
        return cp(st_w.at[k, r, :], (dwq_hbm, dwk_hbm, dwv_hbm)[k].at[r, :], 49 + 4 * k + t)

    o_w1 = cp(st_w1, dw1_hbm, 0)
    o_w2 = cp(st_w2, dw2_hbm, 1)
    o_wo = cp(st_w.at[3], dwo_hbm, 2)
    o_b1 = cp(b1_buf, db1_hbm, 12)
    o_b2 = cp(b2_buf, db2_hbm, 13)
    o_beta = cp(beta_buf, dbeta_hbm, 14)
    o_c = cp(c_buf, dc_hbm, 15)

    def o_mod(k):
        cs = pl.ds(_mo(k * 2 * D, 128), 2 * D)
        return cp(st_mod.at[:, cs], dwmod_hbm.at[:, cs], 6 + k)

    def o_mod01(t):
        r = pl.ds(_mo(t * WCH, 16), WCH)
        return cp(st_mod.at[r, pl.ds(0, 2 * D)], dwmod_hbm.at[r, pl.ds(0, 2 * D)], 17 + t)

    def dsc_pair(j, c_):
        c0 = 2 * j * D
        dm = rowbuf[0:1, pl.ds(_mo(c0, 128), 2 * D)]
        dsc_ref[...] += _dot(jnp.broadcast_to(dm[:, 0:D], (16, D)).astype(bf16),
                             wmod_buf[:, pl.ds(_mo(c0, 128), D)], NT)
        chain = _Chain(j)
        dm8 = rowbuf[:, pl.ds(_mo(c0 + D, 128), D)]
        for r in range(0, D, 32):
            w = wmod_buf[r:r + 32, pl.ds(_mo(c0 + D, 128), D)].astype(f32)
            dmt = jnp.concatenate([chain.tie(dm8[:, n * 128:(n + 1) * 128], 32) for n in range(5)], axis=1)
            a = dscT[r:r + 32, :] + _fold(w * dmt)
            chain.push(_vsum(a))
            dscT[r:r + 32, :] = a
        return c_

    def dmod_pair(j, c_):
        cs = pl.ds(_mo(j * 2 * D, 128), 2 * D)
        dm = rowbuf[0:1, cs]
        for r in range(0, D, 32):
            st_mod[r:r + 32, cs] = (_rep(scT[r:r + 32, :], 2 * D) * dm).astype(bf16)
        o_mod(j).start()
        return c_

    r40 = _iota((40, 128), 0)
    hmask = [jnp.logical_and(r40 >= 10 * j, r40 < 10 * j + 10) for j in range(4)]

    def head_rows(x, j, mask=True):
        parts = []
        for t in range(x.shape[1] // 128):
            y = _rot(x[:, t * 128:(t + 1) * 128], j)
            parts.append(jnp.where(hmask[j][8 * j:8 * j + 16], y, jnp.uint32(0)) if mask else y)
        return jnp.concatenate(parts, axis=1)

    def segment(it, carry):
        s = NSEG - 1 - it
        r0 = _mo(s * (D // 2), 8)
        tok = pl.ds(_mo(s * L, L), L)
        last = it == NSEG - 1
        prev = lambda a: jnp.where(it == 0, 0.0, a)

        def q_part(lo, hi):
            q = _dot(_B(wqoT[lo // 2:hi // 2, :]), _B(h1T[pl.ds(r0, D // 2), :]), NN)
            qT[lo // 2:hi // 2, :] = _pack(q)
            qs = _pack(q * (SCALE * LOG2E))
            for i in range(lo // QR, hi // QR):
                for j in range(4):
                    b = i * 40 - lo // 2 + 8 * j
                    qsT[(4 * i + j) * 16:(4 * i + j + 1) * 16, :] = head_rows(qs[b:b + 16], j)
            pqT[lo // 2:hi // 2, :] = _pack(_phi(q))

        q_part(0, QS)
        r16 = _iota((16, L), 0)

        def build_kv(i):
            k_u = kT[pl.ds(r0 + i * 40, 40), :]
            v_u = vT[pl.ds(r0 + i * 40, 40), :]
            knat[i * 256:(i + 1) * 256, :] = _U(_B(jnp.concatenate([k_u, zeros24], axis=0)).T)
            for j in range(4):
                keep = jnp.logical_and(r16 >= 2 * j, r16 < 2 * j + 10)
                vaug[(4 * i + j) * 16:(4 * i + j + 1) * 16, :] = jnp.where(keep, v_u[8 * j:8 * j + 16], ONES_U)

        def head_w(x, j, aug=None):
            w = [None] * 8
            w[j], w[j + 1] = x[0:8], x[8:16]
            if aug is not None:
                w[5] = aug
            return w

        def score_tile(nat, i, t, u, w):
            b0 = _mo(i * 256 + u * 64, 8)
            zero = jnp.zeros((8, 128), u32)
            tile = lambda bl: jnp.concatenate([zero if x is None else x for x in bl], axis=0)
            w4 = _B(jnp.concatenate([tile(x) for x in w], axis=1))
            if u != t:
                return _dot(_B(nat[pl.ds(b0, 64), :]), w4, NN)
            lo = _iota((8, 128), 1) < 64
            mix = lambda x, y: None if x is None and y is None else jnp.where(
                lo, zero if x is None else x, zero if y is None else y)
            top = _dot(_B(nat[pl.ds(b0, 32), :]), w4, NN)
            w2 = jnp.concatenate([tile([mix(x, y) for x, y in zip(w[j], w[j + 1])]) for j in (0, 2)], axis=1)
            bot = _dot(_B(nat[pl.ds(_mo(b0 + 32, 8), 32), :]), _B(w2), NN)
            bot = jnp.concatenate([bot[:, 0:128], bot[:, 0:128], bot[:, 128:256], bot[:, 128:256]], axis=1)
            return jnp.concatenate([top, bot], axis=0)

        def s_tile(i, t, u, mx):
            qt = qsT[pl.ds(_mo(i * 64, 16), 64), t * 128:(t + 1) * 128]
            sc_ = score_tile(knat, i, t, u, [head_w(qt[16 * j:16 * j + 16], j) for j in range(4)])
            if u == t:
                lane = _iota((128, 128), 1)
                sc_ = jnp.concatenate(
                    [jnp.where(_iota((128, 128), 0) <= (lane if j % 2 else lane ^ 64),
                               sc_[:, j * 128:(j + 1) * 128], -1e30) for j in range(4)], axis=1)
            sbuf[2 * POFF[t] + u * 128:2 * POFF[t] + (u + 1) * 128, :] = sc_
            for k in range(16):
                v = sc_[8 * k:8 * k + 8]
                mx = v if mx is None else jnp.maximum(mx, v)
            if u == t:
                mx = jnp.max(mx, axis=0, keepdims=True)
            return mx

        def p_tile(i, t, u, mx, ws):
            for j in range(4):
                lj = slice(j * 128, (j + 1) * 128)
                sj = sbuf[2 * POFF[t] + u * 128:2 * POFF[t] + (u + 1) * 128, lj]
                p = jnp.exp2(sj - mx[:, lj]).astype(bf16)
                p_ref[pl.ds(_mo(i * 640 + POFF[t] + u * 64, 8), 64), lj] = _U(p)
                va = _B(vaug[pl.ds(_mo((i * 4 + j) * 16, 16), 16), u * 128:(u + 1) * 128])
                w = _dot(va, p, NN)
                ws[j] = w if ws[j] is None else ws[j] + w
            if u == t:
                ws = [_rot(ws[j], j) for j in range(4)]
                ls = [1.0 / (ws[j][24:32] if j < 2 else ws[j][0:8]) for j in range(4)]
                linv = _assemble_rows(ls)
                rq = pl.ds(_mo(i * QR, 8), QR)
                lt = slice(t * 128, (t + 1) * 128)
                ad = _assemble(ws) * linv
                adot[rq, lt] = ad
                g = gT_ref[rq, :]
                cinv[rq, lt] = linv * (1.0 - g)
                o = g * amem[rq, lt] + (1.0 - g) * ad
                oT[pl.ds(_mo(i * 40, 8), 40), lt] = _pack(o)

        mx_first = None
        for i in range(NQ):
            build_kv(i)
            if i == QP2:
                q_part(QS, D)
            if i == QP:
                for u in range(4):
                    mx_first = s_tile(0, 3, u, mx_first)

        def attn_fwd(i, mx3):
            i_next = jnp.minimum(i + 1, NQ - 1)
            mx = {3: mx3, 2: None, 1: None, 0: None, 4: None}
            ws = {t: [None] * 4 for t in range(4)}
            s_jobs = [(2, 0), (2, 1), (2, 2), (1, 0), (1, 1), (0, 0), (4, 0), (4, 1), (4, 2), (4, 3)]
            p_jobs = [(3, 0), (3, 1), (3, 2), (3, 3), (2, 0), (2, 1), (2, 2), (1, 0), (1, 1), (0, 0)]
            def mem_read():
                rq = pl.ds(_mo(i * QR, 8), QR)
                mm = m_state[pl.ds(_mo(s * D + i * QR, 8), QR), :]
                mt = jnp.concatenate([mm, jnp.zeros((48, 128), f32)], axis=0).T
                zh = jnp.where((_iota((32, 128), 0) // 8) == (_iota((32, 128), 1) // DH), mt[QR:QR + 32], 0.0)
                lhs = jnp.concatenate([jnp.where(bd, mt[0:QR], 0.0), zh], axis=0).astype(bf16)
                pq_w = _B(jnp.concatenate([pqT[pl.ds(_mo(i * 40, 8), 40), :], zeros24], axis=0))
                nd = _dot(lhs, pq_w, NN)
                rd = 1.0 / (nd[QR:] + 1e-6)
                rd = _assemble_rows([rd[8 * j:8 * j + 8] for j in range(4)])
                amem[rq, :] = nd[0:QR] * rd
                rden[rq, :] = _rep(gT_ref[rq, :]) * rd

            for n_, ((st, su), (pt, pu)) in enumerate(zip(s_jobs, p_jobs)):
                if n_ == MPOS:
                    mem_read()
                if st == 4:
                    mx[4] = s_tile(i_next, 3, su, mx[4])
                else:
                    mx[st] = s_tile(i, st, su, mx[st])
                p_tile(i, pt, pu, mx[pt], ws[pt])
            return mx[4]

        with _scope("attn_fwd"):
            _loop(NQ, attn_fwd, mx_first, UF)

        dyT[...] = _U(dy_buf[tok, :].T)
        chain = _Chain(it)
        for r in range(0, D, RC):
            gb = modT[5 * D + r:5 * D + r + RC, :]
            gb = jnp.concatenate([chain.tie(gb[0:8], 8), gb[8:]], axis=0)
            dffn = _B(dyT[r // 2:(r + RC) // 2, :]).astype(f32) * _rep(gb)
            dffnT[r // 2:(r + RC) // 2, :] = _pack(dffn)
            db = acc_vec[6 * D + r:6 * D + r + RC, :] + _fold(dffn)
            chain.push(db[0:8])
            acc_vec[6 * D + r:6 * D + r + RC, :] = db
        chain0 = chain
        attn = _dot(_B(wqoT[D // 2:D, :]), _B(oT[...]), NN)
        for t in range(4):
            lt = slice(t * 128, (t + 1) * 128)
            acc = chain0.tie(jnp.zeros((8, 128), f32), 8) if t == TIE0 else None
            for r in range(0, D, RC):
                at = attn[r:r + RC, lt]
                sA[r:r + RC, lt] = at
                x2 = _B(xT[pl.ds(r0 + r // 2, RC // 2), lt]).astype(f32) + modT[2 * D + r:2 * D + r + RC, :] * at
                sB[r:r + RC, lt] = x2
                acc = _vsum(x2, acc)
            mu2 = jnp.sum(acc, axis=0, keepdims=True) * (1.0 / D)
            accs = [None] * (1 if t < 3 else 4)
            for n, r in enumerate(range(0, D, RC)):
                xc2 = sB[r:r + RC, lt] - mu2
                accs[n % len(accs)] = _vsum(xc2 * xc2, accs[n % len(accs)])
            acc = _vsum(jnp.concatenate(accs, axis=0))
            rstd2 = jax.lax.rsqrt(jnp.sum(acc, axis=0, keepdims=True) * (1.0 / D) + EPS)
            stat2[:, lt] = jnp.broadcast_to(rstd2, (8, 128))
            mu2 = jnp.broadcast_to(mu2, (8, 128))
            chain = _Chain(it, 1 if t < 3 else LAGT)
            for r in range(0, D, RC):
                xh2 = (sB[r:r + RC, lt] - chain.tie(mu2, RC)) * rstd2
                sC[r:r + RC, lt] = xh2
                h2 = xh2 * modT[4 * D + r:4 * D + r + RC, :] + modT[3 * D + r:3 * D + r + RC, :]
                chain.push(h2)
                h2T[r // 2:(r + RC) // 2, lt] = _pack(h2)

        def ffn_chunk(ci, c_):
            rp = pl.ds(_mo(ci * (FCH // 2), 8), FCH // 2)
            rf = pl.ds(_mo(ci * FCH, 16), FCH)
            h2b = _B(h2T[...])
            dfb = _B(dffnT[...])
            u = _dot(w1_buf[rf, :], h2b, NN) + _rep(b1T[rf, :])
            dg = _dot(w2_buf[rf, :], dfb, NN)
            u2 = u * u
            th = jnp.tanh(u * (GELU_C1 + GELU_C2 * u2))
            hp = 0.5 * th + 0.5
            gactT[rp, :] = _pack(u * hp)
            gp = hp + (0.5 * u) * (1.0 - th * th) * (GELU_C1 + (3.0 * GELU_C2) * u2)
            du = dg * gp
            duT[rp, :] = _pack(du)
            acc_vec[pl.ds(_mo(7 * D + ci * FCH, 8), FCH), :] += _fold(du)
            a2 = prev(acc_w2[rf, :]) + _dot(_B(gactT[rp, :]), dfb, NT)
            acc_w2[rf, :] = a2
            st_w2[rf, :] = a2.astype(bf16)
            a1 = prev(acc_w1T[rf, :]) + _dot(_B(duT[rp, :]), h2b, NT)
            acc_w1T[rf, :] = a1
            st_w1[rf, :] = a1.astype(bf16)
            for blk in (ci, ci + NFC, jnp.minimum(ci + 2 * NFC, FP // 128 - 1)):
                rb = pl.ds(_mo(blk * 128, 128), 128)
                w1N[:, rb] = _U(w1_buf[rb, :].T)
                w2T[:, rb] = _U(w2_buf[rb, :].T)
            for i in (ci, jnp.minimum(ci + NFC, NQ - 1)):
                v_u = vT[pl.ds(_mo(r0 + i * 40, 8), 40), :]
                vnat[pl.ds(_mo(i * 256, 256), 256), :] = _U(_B(jnp.concatenate([v_u, ones24], axis=0)).T)
            return c_

        with _scope("ffn_chunk"):
            _loop(NFC, ffn_chunk, 0, UC)

        @pl.when(last)
        def _():
            o_w1.start()
            o_w2.start()

        def post_ffn(hf, c_):
            hl = pl.ds(_mo(hf * HL, HL), HL)
            rows = pl.ds(_mo(s * L + hf * HL, HL), HL)
            dh2 = _dot(_B(w1N[...]), _B(duT[:, hl]), NN)
            for t in range(2):
                lt = pl.ds(_mo(hf * HL + t * 128, 128), 128)
                s1 = s2 = None
                for r in range(0, D, RC):
                    dh = dh2[r:r + RC, t * 128:(t + 1) * 128]
                    xh2 = sC[r:r + RC, lt]
                    acc_vec[3 * D + r:3 * D + r + RC, :] += dh
                    acc_vec[4 * D + r:4 * D + r + RC, :] += dh * xh2
                    dxh = dh * modT[4 * D + r:4 * D + r + RC, :]
                    sD[r:r + RC, lt] = dxh
                    s1 = _vsum(dxh, s1)
                    s2 = _vsum(dxh * xh2, s2)
                m1 = jnp.sum(s1, axis=0, keepdims=True) * (1.0 / D)
                m2 = jnp.sum(s2, axis=0, keepdims=True) * (1.0 / D)
                rs = stat2[0:1, lt]
                m1 = jnp.broadcast_to(m1, (8, 128))
                chain = _Chain(hf)
                for r in range(0, D, RC):
                    dx2 = _B(dyT[r // 2:(r + RC) // 2, lt]).astype(f32) + rs * (
                        sD[r:r + RC, lt] - chain.tie(m1, RC) - sC[r:r + RC, lt] * m2)
                    chain.push(dx2)
                    sD[r:r + RC, lt] = dx2
                    acc_vec[2 * D + r:2 * D + r + RC, :] += dx2 * sA[r:r + RC, lt]
                    dffnT[r // 2:(r + RC) // 2, lt] = _pack(dx2 * modT[2 * D + r:2 * D + r + RC, :])

            def ffn_part(lo, hi):
                ffn = _dot(_B(w2T[lo // 2:hi // 2, :]), _B(gactT[:, hl]), NN) + _rep(b2T[lo:hi, :], HL)
                acc_vec[5 * D + lo:5 * D + hi, :] += _fold(_B(dyT[lo // 2:hi // 2, hl]).astype(f32) * ffn)
                outT = sB[lo:hi, hl] + _rep(modT[5 * D + lo:5 * D + hi, :], HL) * ffn
                x_buf[rows, lo:hi] = outT.astype(bf16).T

            ffn_part(0, _FSPLIT)
            do_all = _dot(wqkv_buf[3], _B(dffnT[:, hl]), NN)
            if _FSPLIT < D:
                ffn_part(_FSPLIT, D)
            for i in range(NQ):
                rq = slice(i * QR, (i + 1) * QR)
                do = do_all[rq]
                ad = adot[rq, hl]
                am = amem[rq, hl]
                acc_vec[10 * D + i * QR:10 * D + (i + 1) * QR, :] += _fold(do * (am - ad))
                dop = _pack(do * cinv[rq, hl])
                parts = _head_partials(_B(dop).astype(f32) * ad)
                for j in range(4):
                    hi = (-parts[j]).astype(bf16).astype(f32)
                    lo = -parts[j] - hi
                    b = i * 96 + 24 * j
                    dOp[b:b + 16, hl] = head_rows(dop[8 * j:8 * j + 16], j)
                    dOp[b + 16:b + 24, hl] = head_rows(_pack(jnp.concatenate([hi, lo], axis=0)), j, False)
                dnum = do * rden[rq, hl]
                tp = _head_partials(dnum * am)
                wmemT[i * 56:(i + 1) * 56, hl] = _pack(jnp.concatenate([dnum] + [-x for x in tp], axis=0))
            out_copy(s, hf).start()
            return c_

        with _scope("post_ffn"):
            jax.lax.fori_loop(0, 2, post_ffn, 0)

        def attn_bwd(i, c_):
            rq = pl.ds(_mo(i * QR, 8), QR)
            rp = pl.ds(_mo(i * 40, 8), 40)
            d0 = _mo(i * 96, 8)
            dq = [[None] * 4 for _ in range(4)]
            dk = [[None] * 4 for _ in range(4)]
            dv = [[None] * 4 for _ in range(4)]
            mem = {}

            def wmem():
                return _B(jnp.concatenate([wmemT[pl.ds(_mo(i * 56, 8), 56), :], jnp.zeros((8, L), u32)], axis=0))

            def mem_dq():
                mm = m_state[pl.ds(_mo(s * D + i * QR, 8), QR), :]
                dpq = _dot(jnp.where(mask2, mm, 0.0).astype(bf16), wmem(), NN)
                qq = _B(qT[rp, :]).astype(f32)
                mem['q'] = dpq * jnp.where(qq > 0, 1.0, _B(pqT[rp, :]).astype(f32))

            def mem_dkv():
                kk = _B(kT[pl.ds(r0 + i * 40, 40), :]).astype(f32)
                pk = _phi(kk)
                pk_w = jnp.concatenate([pk, jnp.zeros((48, L), f32)], axis=0).astype(bf16)
                v_aug = _B(jnp.concatenate([vT[pl.ds(r0 + i * 40, 40), :], ones24], axis=0))
                dms = dm_state[rq, :]
                dpk = _dot(jnp.where(mask2, dms, 0.0).astype(bf16), v_aug, NN)
                dmt = jnp.concatenate([jnp.where(bd, dms, 0.0), jnp.zeros((48, 128), f32)], axis=0).T
                mem['v'] = _dot(dmt[0:QR].astype(bf16), pk_w, NN)
                mem['k'] = dpk * jnp.where(kk > 0, 1.0, pk)

            def mem_update():
                dm_state[rq, :] += _dot(_B(pqT[rp, :]), wmem(), NT)

            def dp_tile(t, u):
                lt = slice(t * 128, (t + 1) * 128)
                dt = dOp[pl.ds(d0, 96), lt]
                wd = [head_w(dt[24 * j:24 * j + 16], j, dt[24 * j + 16:24 * j + 24]) for j in range(4)]
                dp = score_tile(vnat, i, t, u, wd)
                res = []
                for j in range(4):
                    p = _B(p_ref[pl.ds(_mo(i * 640 + POFF[t] + u * 64, 8), 64), j * 128:(j + 1) * 128])
                    res.append((dp[:, j * 128:(j + 1) * 128] * p.astype(f32)).astype(bf16))
                return res

            def thin_tile(t, u, ds):
                lt = slice(t * 128, (t + 1) * 128)
                for j in range(4):
                    p = _B(p_ref[pl.ds(_mo(i * 640 + POFF[t] + u * 64, 8), 64), j * 128:(j + 1) * 128])
                    kw = _B(kT[pl.ds(r0 + i * 40 + 8 * j, 16), u * 128:(u + 1) * 128])
                    qw = _B(qsT[pl.ds(_mo(i * 64 + 16 * j, 16), 16), lt])
                    dw = _B(dOp[pl.ds(d0 + 24 * j, 16), lt])
                    b = _dot(dw, p, NT)
                    a = _dot(qw, ds[j], NT)
                    e = _dot(kw, ds[j], NN)
                    dq[j][t] = e if dq[j][t] is None else dq[j][t] + e
                    dk[j][u] = a if dk[j][u] is None else dk[j][u] + a
                    dv[j][u] = b if dv[j][u] is None else dv[j][u] + b
                if u == t:
                    col = lambda w: _assemble([w[j][t] for j in range(4)])
                    for j in range(4):
                        dq[j][t] = _rot(dq[j][t], j)
                    dqkvT[rp, lt] = _pack(col(dq) * SCALE + mem['q'][:, lt])
                    dqkvT[pl.ds(_mo(D // 2 + i * 40, 8), 40), lt] = _pack(col(dk) * (1.0 / LOG2E) + mem['k'][:, lt])
                    dqkvT[pl.ds(_mo(D + i * 40, 8), 40), lt] = _pack(col(dv) + mem['v'][:, lt])

            jobs = [(t, u) for t in (3, 2, 1, 0) for u in range(t + 1)]
            def dwo(n):
                def f():
                    cs = slice(n * 128, (n + 1) * 128)
                    r16 = pl.ds(_mo(i * QR, 16), QR)
                    ao = prev(acc_wo[rq, cs]) + _dot(_B(oT[rp, :]), _B(dffnT[n * 64:(n + 1) * 64, :]), NT)
                    acc_wo[rq, cs] = ao
                    st_w[3, r16, cs] = ao.astype(bf16)
                return f

            def rowsums():
                rowbuf[:, pl.ds(_mo(2 * D + i * D, 128), D)] = jnp.broadcast_to(
                    _rowsum(acc_vec[pl.ds(_mo(2 * D + i * D, 8), D), :]), (8, D))

            extra = {0: [mem_dq], 1: [mem_dkv], 9: [mem_update]}
            extra.setdefault(RSP, []).append(rowsums)
            for n, pos in enumerate(_DWO_POS):
                extra.setdefault(pos, []).append(dwo(n))
            for f in extra.get(-1, []):
                f()
            ds = dp_tile(*jobs[0])
            for n_, job in enumerate(jobs):
                ds_next = dp_tile(*jobs[n_ + 1]) if n_ + 1 < len(jobs) else None
                for f in extra.get(n_, []):
                    f()
                thin_tile(job[0], job[1], ds)
                ds = ds_next
            for f in extra.get(10, []):
                f()
            return c_

        with _scope("attn_bwd"):
            _loop(NQ, attn_bwd, 0, UB)

        @pl.when(last)
        def _():
            o_wo.start()
            b2_buf[...] = rowbuf[0:1, 6 * D:7 * D].reshape(D).astype(bf16)
            o_b2.start()
            b1_buf[...] = rowbuf[0:1, 7 * D:7 * D + F].reshape(F).astype(bf16)
            o_b1.start()
            jax.lax.fori_loop(1, 3, dmod_pair, 0)

        def dw_chunk(t):
            ra = pl.ds(_mo(t * WCH, 16), WCH)
            aw = prev(acc_wqkv[ra, :]) + _dot(_B(h1T[pl.ds(r0 + t * (WCH // 2), WCH // 2), :]), _B(dqkvT[...]), NT)
            acc_wqkv[ra, :] = aw
            for k in range(3):
                st_w[k, ra, :] = aw[:, k * D:(k + 1) * D].astype(bf16)

            @pl.when(last)
            def _():
                for k in range(3):
                    o_w(k, t).start()

        def qkv_bwd_a(a, c_):
            hl = pl.ds(_mo(a * HL, HL), HL)
            dh1 = _dot(wqkv_buf[0], _B(dqkvT[0:D // 2, hl]), NN)
            dh1 = dh1 + _dot(wqkv_buf[1], _B(dqkvT[D // 2:D, hl]), NN)
            dh1 = dh1 + _dot(wqkv_buf[2], _B(dqkvT[D:3 * D // 2, hl]), NN)
            for t in range(2):
                lt = pl.ds(_mo(a * HL + t * 128, 128), 128)
                mu = stat1[pl.ds(_mo(s * 16, 8), 1), lt]
                rstd = stat1[pl.ds(_mo(s * 16 + 8, 8), 1), lt]
                xh = lambda r: (_B(xT[pl.ds(r0 + r // 2, RC // 2), lt]).astype(f32) - mu) * rstd
                s1 = s2 = None
                for r in range(0, D, RC):
                    dh = dh1[r:r + RC, t * 128:(t + 1) * 128]
                    xh1 = xh(r)
                    acc_vec[r:r + RC, :] += dh
                    acc_vec[D + r:D + r + RC, :] += dh * xh1
                    dxh = dh * modT[D + r:D + r + RC, :]
                    sA[r:r + RC, lt] = dxh
                    s1 = _vsum(dxh, s1)
                    s2 = _vsum(dxh * xh1, s2)
                m1 = jnp.broadcast_to(jnp.sum(s1, axis=0, keepdims=True) * (1.0 / D), (8, 128))
                m2 = jnp.sum(s2, axis=0, keepdims=True) * (1.0 / D)
                chain = _Chain(a)
                for r in range(0, D, RC):
                    dx = _pack(sD[r:r + RC, lt] + rstd * (sA[r:r + RC, lt] - chain.tie(m1, RC) - xh(r) * m2))
                    chain.push(pltpu.bitcast(dx, f32))
                    dyT[r // 2:(r + RC) // 2, lt] = dx
                dy_buf[pl.ds(_mo(s * L + a * HL + t * 128, 128), 128), :] = _B(dyT[:, lt]).T
            dw_chunk(a)
            dx_copy(s, a).start()
            return c_

        def qkv_bwd_b(b, c_):
            dw_chunk(2 + b)
            return c_

        with _scope("qkv_bwd_a"):
            jax.lax.fori_loop(0, 2, qkv_bwd_a, 0)

        @pl.when(last)
        def _():
            dm = _rowsum(acc_vec[0:2 * D, :])

            def piece(t, c_):
                r = pl.ds(_mo(t * WCH, 16), WCH)
                st_mod[r, 0:2 * D] = (_rep(scT[r, :], 2 * D) * dm).astype(bf16)
                o_mod01(t).start()
                return c_

            jax.lax.fori_loop(0, 4, piece, 0)
            rowbuf[:, 0:2 * D] = jnp.broadcast_to(dm, (8, 2 * D))

        with _scope("qkv_bwd_b"):
            jax.lax.fori_loop(0, 2, qkv_bwd_b, 0)

        return carry

    with _scope("segment"):
        jax.lax.fori_loop(0, NSEG, segment, 0)

    gate = gate_row()
    dgc = jnp.sum(acc_vec[10 * D:11 * D, :], axis=1, keepdims=True)
    dgate = jnp.sum(jnp.where(head_onehot(), jnp.broadcast_to(dgc, (D, H)), 0.0), axis=0, keepdims=True)
    beta_buf[...] = (dgate * gate * (1.0 - gate)).reshape(H).astype(bf16)
    o_beta.start()
    jax.lax.fori_loop(0, 3, dsc_pair, 0)
    c_, sig = silu_parts()
    dsc = dsc_ref[0:1, :] + _rowsum(dscT[...])
    c_buf[...] = (dsc * (sig * (1.0 + c_ * (1.0 - sig)))).astype(bf16)
    o_c.start()

    with _scope("wait1"):
        for s in range(NSEG):
            for hf in range(2):
                out_copy(s, hf).wait()
                dx_copy(s, hf).wait()
        for d in [o_w2, o_w1, o_wo, o_b1, o_b2] + [o_mod(k) for k in range(1, 3)] + [
                o_w(k, t) for k in range(3) for t in range(4)]:
            d.wait()
    with _scope("wait2"):
        o_mod01(0).wait()
        o_mod01(1).wait()
    with _scope("wait3"):
        o_mod01(2).wait()
        o_mod01(3).wait()
    with _scope("wait4"):
        o_c.wait()
        o_beta.wait()


@jax.jit
def pallas_adaLN_cond__memory_aug_infini_attn__dense_activation_gelu__prompt_kernel(
    A_x: jax.Array,
    A_wq: jax.Array,
    A_wk: jax.Array,
    A_wv: jax.Array,
    A_wo: jax.Array,
    A_beta: jax.Array,
    B_x: jax.Array,
    B_w1: jax.Array,
    B_b1: jax.Array,
    B_w2: jax.Array,
    B_b2: jax.Array,
    c: jax.Array,
    w_mod: jax.Array,
    grad_out: jax.Array,
):
    del B_x
    hbm = pl.BlockSpec(memory_space=pltpu.HBM)
    sds = jax.ShapeDtypeStruct
    V = pltpu.VMEM
    scratch = [
        V((S, D), bf16), V((S, D), bf16), V((4, D, D), bf16), V((FP, D), bf16),
        V((FP, D), bf16), V((D, 6 * D), bf16),
        V((H,), bf16), V((F,), bf16), V((D,), bf16), V((1, D), bf16),
        V((F, D), bf16), V((F, D), bf16), V((4, D, D), bf16),
        V((D, D), u32), V((D, D), u32), V((D // 2, FP), u32), V((D // 2, FP), u32),
        V((8 * D, 128), f32), V((F, 128), f32), V((D, 128), f32), V((D, 128), f32), V((D, 128), f32),
        V((16, D), f32), V((D, 128), f32), V((D, 6 * D), bf16),
        V((NSEG * D // 2, L), u32), V((D // 2, L), u32), V((NSEG * 16, L), f32),
        V((NSEG * D // 2, L), u32), V((NSEG * D // 2, L), u32),
        V((NSEG * D // 2, L), u32), V((8, L), f32),
        V(((NSEG + 1) * D, 128), f32), V((D, 128), f32),
        V((D // 2, L), u32), V((H * 16, L), u32), V((D // 2, L), u32),
        V((NQ * 256, 128), u32), V((NQ * 256, 128), u32), V((H * 16, L), u32), V((NQ * 640, L), u32), V((1280, L), f32),
        V((D, L), f32), V((D, L), f32), V((D, L), f32), V((D, L), f32), V((D // 2, L), u32),
        V((D, L), f32), V((D, L), f32), V((D, L), f32), V((D, L), f32),
        V((D // 2, L), u32), V((D // 2, L), u32), V((D // 2, L), u32), V((FP // 2, L), u32), V((FP // 2, L), u32),
        V((NQ * 96, L), u32), V((NQ * 56, L), u32), V((3 * D // 2, L), u32),
        V((D, 3 * D), f32), V((D, D), f32), V((F, D), f32), V((F, D), f32), V((11 * D, 128), f32),
        V((8, 10 * D), f32),
        pltpu.SemaphoreType.DMA((61,)),
    ]
    outs = pl.pallas_call(
        _kernel,
        in_specs=[hbm] * 13,
        out_specs=[hbm] * 13,
        out_shape=[
            sds((1, S, D), bf16), sds((1, S, D), bf16), sds((D, D), bf16), sds((D, D), bf16),
            sds((D, D), bf16), sds((D, D), bf16), sds((H,), bf16), sds((F, D), bf16), sds((F,), bf16),
            sds((F, D), bf16), sds((D,), bf16), sds((1, D), bf16), sds((D, 6 * D), bf16),
        ],
        scratch_shapes=scratch,
        compiler_params=pltpu.CompilerParams(vmem_limit_bytes=124 * 1024 * 1024),
    )(A_x, A_wq, A_wk, A_wv, A_wo, A_beta, B_w1.T, B_b1, B_w2, B_b2, c, w_mod, grad_out)
    out, dx, dwq, dwk, dwv, dwo, dbeta, dw1, db1, dw2, db2, dc, dwmod = outs
    return (out, dx, dwq, dwk, dwv, dwo, dbeta, dw1.T, db1, dw2, db2, dc, dwmod)
```
